```python
import jax
import jax.numpy as jnp

def _softmax(x, axis=-1):
    return jax.nn.softmax(x, axis=axis)
def _gelu(x):
    return jax.nn.gelu(x, approximate=True)
def _silu(x):
    return jax.nn.silu(x)
def _sigmoid(x):
    return jax.nn.sigmoid(x)
def _layernorm(x, axis=-1, eps=1e-5):
    m = jnp.mean(x, axis=axis, keepdims=True)
    v = jnp.var(x, axis=axis, keepdims=True)
    return (x - m) / jnp.sqrt(v + eps)
def _scatter_add(tgt, idx, src, axis=0):
    return tgt.at[idx].add(src)
def _segment_sum(src, seg, n):
    return jax.ops.segment_sum(src, seg, n)
class _Rng:
    def __init__(self, key):
        self._k = key
    def _next(self):
        self._k, sub = jax.random.split(self._k)
        return sub
    def normal(self, shape):
        return jax.random.normal(self._next(), shape, dtype=jnp.bfloat16)
    def randint(self, lo, hi, shape):
        return jax.random.randint(self._next(), shape, lo, hi, dtype=jnp.int32)
    def uniform(self, shape, lo=0.0, hi=1.0):
        return jax.random.uniform(self._next(), shape, jnp.bfloat16, lo, hi)
    def permutation(self, n):
        return jax.random.permutation(self._next(), n)


kernel_name = 'interleave_layers__sliding_block_cached__mixer_s_mlp__decode'

def setup_inputs():
    _rng = _Rng(jax.random.key(int.from_bytes(__import__("os").urandom(4), "little")))
    _w = (lambda a: (lambda t: t.astype(jnp.bfloat16) if jnp.issubdtype(t.dtype, jnp.floating) else t)(jnp.asarray(a)))
    def _A_setup():
        B, Sq, D = 1, 1, 640
        Hq, Hkv, Sk, Dh = 32, 32, 32768, 192
        assert Hq % Hkv == 0, (Hq, Hkv)
        return {
            "x": _w((lambda *s: _rng.normal(s) * 0.05)(B, Sq, D)),
            "k_cache": _w((lambda *s: _rng.normal(s) * 0.05)(B, Hkv, Sk, Dh)),
            "v_cache": _w((lambda *s: _rng.normal(s) * 0.05)(B, Hkv, Sk, Dh)),
            "wq": _w((lambda *s: _rng.normal(s) * 0.05)(D, Hq * Dh) * (D ** -0.5)),
            "wo": _w((lambda *s: _rng.normal(s) * 0.05)(Hq * Dh, D) * ((Hq * Dh) ** -0.5)),
        }
    _A_in = _A_setup()

    def _B_setup():
        B, S, D, F = 1, 1, 640, 1536
        return {
            "x":  _w((lambda *s: _rng.normal(s) * 0.05)(B, S, D)),
            "w1": _w((lambda *s: _rng.normal(s) * 0.05)(D, D) * (D ** -0.5)),
            "w2": _w((lambda *s: _rng.normal(s) * 0.05)(D, D) * (D ** -0.5)),
            "w3": _w((lambda *s: _rng.normal(s) * 0.05)(D, F) * (D ** -0.5)),
            "w4": _w((lambda *s: _rng.normal(s) * 0.05)(F, D) * (F ** -0.5)),
        }
    _B_in = _B_setup()

    return {
        "A_x": _A_in["x"],
        "A_k_cache": _A_in["k_cache"],
        "A_v_cache": _A_in["v_cache"],
        "A_wq": _A_in["wq"],
        "A_wo": _A_in["wo"],
        "B_x": _B_in["x"],
        "B_w1": _B_in["w1"],
        "B_w2": _B_in["w2"],
        "B_w3": _B_in["w3"],
        "B_w4": _B_in["w4"],
    }

def reference(A_x, A_k_cache, A_v_cache, A_wq, A_wo, B_x, B_w1, B_w2, B_w3, B_w4):
    def _A_ref(x, k_cache, v_cache, wq, wo):
        B, Sq, D = x.shape
        Hq, Dh = 32, 192
        Hkv, Sk = k_cache.shape[1], k_cache.shape[2]
        W = min(4096, max(256, Sk // 4))
        rep = Hq // Hkv
        q = (lambda x, *d: x.transpose(*d))((x @ wq).reshape(B, Sq, Hq, Dh), 0, 2, 1, 3)
        k = jnp.repeat(k_cache[:, :, Sk - W:, :], rep, axis=1)
        v = jnp.repeat(v_cache[:, :, Sk - W:, :], rep, axis=1)
        scores = jnp.einsum("bhqd,bhkd->bhqk", q, k) * (Dh ** -0.5)
        p = _softmax(scores, axis=-1)
        o = jnp.einsum("bhqk,bhkd->bhqd", p, v)
        return (lambda x, *d: x.transpose(*d))(o, 0, 2, 1, 3).reshape(B, Sq, Hq * Dh) @ wo

    def _B_ref(x, w1, w2, w3, w4):
        B, S, D = x.shape
        h = _gelu(_layernorm(x, axis=-1) @ w1)
        c = D // 4
        g0 = jnp.pad(h[:, :, 0*c:1*c], ((0, 0), (1, 0), (0, 0)))[:, :S, :]
        g1 = jnp.pad(h[:, :, 1*c:2*c], ((0, 0), (0, 1), (0, 0)))[:, 1:, :]
        g2 = jnp.pad(h[:, :, 2*c:3*c], ((0, 0), (2, 0), (0, 0)))[:, :S, :]
        g3 = jnp.pad(h[:, :, 3*c:   ], ((0, 0), (0, 2), (0, 0)))[:, 2:, :]
        hs = jnp.concatenate([g0, g1, g2, g3], axis=-1) @ w2
        x1 = x + hs
        h2 = _gelu(_layernorm(x1, axis=-1) @ w3) @ w4
        return x1 + h2

    x = A_x
    x = x + _A_ref(_layernorm(x, axis=-1), A_k_cache, A_v_cache, A_wq, A_wo)
    x = x + _B_ref(_layernorm(x, axis=-1), B_w1, B_w2, B_w3, B_w4)
    x = x + _A_ref(_layernorm(x, axis=-1), A_k_cache, A_v_cache, A_wq, A_wo)
    x = x + _B_ref(_layernorm(x, axis=-1), B_w1, B_w2, B_w3, B_w4)
    return x
```

```python
import functools
import jax
import jax.numpy as jnp
import numpy as np
from jax import lax
import jax.experimental.pallas as pl
import jax.experimental.pallas.tpu as pltpu

H, DH, SK, W, D, F = 32, 192, 32768, 4096, 640, 1536
HD = H * DH
G = 8
NG = H // G
GR = G * DH
M = 8
EPS = 1e-5
SCALE = DH ** -0.5


def _ln(x):
    m = jnp.mean(x, axis=-1, keepdims=True)
    xc = x - m
    v = jnp.mean(xc * xc, axis=-1, keepdims=True)
    return xc / jnp.sqrt(v + EPS)


def _gelu(x):
    c = np.float32(np.sqrt(2.0 / np.pi))
    return 0.5 * x * (1.0 + jnp.tanh(c * (x + 0.044715 * (x * x * x))))


def _dot(a, b):
    return jnp.dot(a, b, preferred_element_type=jnp.float32)


def _dot_nt(a, b):
    return lax.dot_general(a, b, (((1,), (1,)), ((), ())), preferred_element_type=jnp.float32)


def kernel(x_ref, k_hbm, v_hbm, wq_hbm, wo_hbm, w3_hbm, w4_hbm, o_ref,
           kb, vb, wq, wo, w3, w4, sems):
    copies = [pltpu.make_async_copy(wq_hbm, wq, sems.at[0]),
              pltpu.make_async_copy(wo_hbm, wo, sems.at[1])]
    for g in range(NG):
        copies.append(pltpu.make_async_copy(
            k_hbm.at[pl.ds(g * GR, GR), pl.ds(SK - W, W)], kb.at[g], sems.at[2 + 2 * g]))
        copies.append(pltpu.make_async_copy(
            v_hbm.at[pl.ds(g * GR, GR), pl.ds(SK - W, W)], vb.at[g], sems.at[3 + 2 * g]))
    copies.append(pltpu.make_async_copy(w3_hbm, w3, sems.at[2 + 2 * NG]))
    copies.append(pltpu.make_async_copy(w4_hbm, w4, sems.at[3 + 2 * NG]))
    DEPTH = 3
    for c in copies[:DEPTH]:
        c.start()
    state = {"n": 0}

    def wait_next():
        i = state["n"]
        copies[i].wait()
        if i + DEPTH < len(copies):
            copies[i + DEPTH].start()
        state["n"] = i + 1

    row = lax.broadcasted_iota(jnp.int32, (M, GR), 0)
    col = lax.broadcasted_iota(jnp.int32, (M, GR), 1)
    blk = (col >= row * DH) & (col < row * DH + DH)

    x = jnp.broadcast_to(x_ref[0].astype(jnp.float32), (M, D))

    for p in range(2):
        first = p == 0
        xn = _ln(x).astype(jnp.bfloat16)
        if first:
            wait_next()
            wait_next()
        q = _dot(xn, wq[...])
        acc = jnp.zeros((M, D), jnp.float32)
        for g in range(NG):
            qb = jnp.where(blk, q[:, g * GR:(g + 1) * GR], 0.0).astype(jnp.bfloat16)
            if first:
                wait_next()
            s = _dot(qb, kb[g])
            m = jnp.max(s, axis=-1, keepdims=True)
            e = jnp.exp((s - m) * SCALE)
            l = jnp.sum(e, axis=-1, keepdims=True)
            if first:
                wait_next()
            o = _dot_nt(e.astype(jnp.bfloat16), vb[g])
            o = jnp.where(blk, o / l, 0.0).astype(jnp.bfloat16)
            acc = acc + _dot(o, wo[g * GR:(g + 1) * GR, :])
        x = x + jnp.sum(acc, axis=0, keepdims=True)
        x1 = _ln(x)
        h = _ln(x1).astype(jnp.bfloat16)
        if first:
            wait_next()
        h = _gelu(_dot(h, w3[...])).astype(jnp.bfloat16)
        if first:
            wait_next()
        x = x + x1 + _dot(h, w4[...])
    o_ref[0] = x[0:1, :].astype(o_ref.dtype)


@jax.jit
def pallas_interleave_layers__sliding_block_cached__mixer_s_mlp__decode_kernel(
    A_x, A_k_cache, A_v_cache, A_wq, A_wo, B_x, B_w1, B_w2, B_w3, B_w4,
):
    del B_x, B_w1, B_w2
    kt = jnp.swapaxes(A_k_cache, 2, 3).reshape(HD, SK)
    vt = jnp.swapaxes(A_v_cache, 2, 3).reshape(HD, SK)
    hbm = pl.BlockSpec(memory_space=pltpu.HBM)
    return pl.pallas_call(
        kernel,
        out_shape=jax.ShapeDtypeStruct((1, 1, D), jnp.bfloat16),
        in_specs=[pl.BlockSpec(memory_space=pltpu.VMEM)] + [hbm] * 6,
        out_specs=pl.BlockSpec(memory_space=pltpu.VMEM),
        scratch_shapes=[
            pltpu.VMEM((NG, GR, W), jnp.bfloat16),
            pltpu.VMEM((NG, GR, W), jnp.bfloat16),
            pltpu.VMEM((D, HD), jnp.bfloat16),
            pltpu.VMEM((HD, D), jnp.bfloat16),
            pltpu.VMEM((D, F), jnp.bfloat16),
            pltpu.VMEM((F, D), jnp.bfloat16),
            pltpu.SemaphoreType.DMA((4 + 2 * NG,)),
        ],
        compiler_params=pltpu.CompilerParams(vmem_limit_bytes=126 * 1024 * 1024),
    )(A_x, kt, vt, A_wq, A_wo, B_w3, B_w4)
```

```python
import functools
import jax
import jax.numpy as jnp
import numpy as np
from jax import lax
import jax.experimental.pallas as pl
import jax.experimental.pallas.tpu as pltpu

H, DH, SK, W, D, F = 32, 192, 32768, 4096, 640, 1536
HD = H * DH
G = 8
NG = H // G
GR = G * DH
M = 8
T = 128
EPS = 1e-5
SCALE = DH ** -0.5


def _ln(x):
    m = jnp.mean(x, axis=-1, keepdims=True)
    xc = x - m
    v = jnp.mean(xc * xc, axis=-1, keepdims=True)
    return xc / jnp.sqrt(v + EPS)


def _gelu(x):
    c = np.float32(np.sqrt(2.0 / np.pi))
    return 0.5 * x * (1.0 + jnp.tanh(c * (x + 0.044715 * (x * x * x))))


def _dot(a, b):
    return jnp.dot(a, b, preferred_element_type=jnp.float32)


def _mm(a, tile, nk, nn):
    outs = [None] * nn
    for k in range(nk):
        ak = a[:, k * T:(k + 1) * T]
        for n in range(nn):
            d = _dot(ak, tile(k, n))
            outs[n] = d if outs[n] is None else outs[n] + d
    return jnp.concatenate(outs, axis=1)


def _mm_n(a, tile, nk, nn):
    outs = []
    for n in range(nn):
        acc = None
        for k in range(nk):
            d = _dot(a[:, k * T:(k + 1) * T], tile(k, n))
            acc = d if acc is None else acc + d
        outs.append(acc)
    return jnp.concatenate(outs, axis=1)


def kernel(x_ref, k_hbm, v_hbm, wq_hbm, wo_hbm, w3_hbm, w4_hbm, o_ref,
           kb, vb, wq, wo, w3, w4, qs, sems):
    def kv_copy(hbm, buf, g, s):
        return pltpu.make_async_copy(
            hbm.at[pl.ds(g * GR, GR), pl.ds(SK - W, W)], buf.at[g], sems.at[s + 2 * g])

    wq_cp = pltpu.make_async_copy(wq_hbm, wq, sems.at[0])
    wo_cp = pltpu.make_async_copy(wo_hbm, wo, sems.at[1])
    w3_cp = pltpu.make_async_copy(w3_hbm, w3, sems.at[2 + 2 * NG])
    w4_cp = pltpu.make_async_copy(w4_hbm, w4, sems.at[3 + 2 * NG])
    wq_cp.start()
    wo_cp.start()
    for g in range(NG):
        kv_copy(v_hbm, vb, g, 2).start()
        kv_copy(k_hbm, kb, g, 3).start()
    w3_cp.start()
    w4_cp.start()

    row = lax.broadcasted_iota(jnp.int32, (M, GR), 0)
    col = lax.broadcasted_iota(jnp.int32, (M, GR), 1)
    blk = (col >= row * DH) & (col < row * DH + DH)

    x0 = jnp.broadcast_to(x_ref[0].astype(jnp.float32), (M, D))

    def one_pass(p, x):
        first = p == 0
        xn = _ln(x).astype(jnp.bfloat16)

        @pl.when(first)
        def _():
            wq_cp.wait()
            wo_cp.wait()

        for g in range(NG):
            q = _mm(xn, lambda k, n: wq[k * T:(k + 1) * T, g * GR + n * T:g * GR + (n + 1) * T], D // T, GR // T)
            qs[g] = jnp.where(blk, q, 0.0)

        def group(g, acc):
            @pl.when(first)
            def _():
                kv_copy(v_hbm, vb, g, 2).wait()

                def tr(j, c):
                    r = pl.multiple_of(j * T, T)
                    for i in range(W // T):
                        b = vb.at[g, pl.ds(r, T), i * T:(i + 1) * T]
                        b[...] = b[...].T
                    return c
                lax.fori_loop(0, GR // T, tr, 0)
                kv_copy(k_hbm, kb, g, 3).wait()

            qb = qs[g].astype(jnp.bfloat16)
            s = _mm(qb, lambda k, n: kb[g, k * T:(k + 1) * T, n * T:(n + 1) * T], GR // T, W // T)
            m = jnp.max(s, axis=-1, keepdims=True)
            e = jnp.exp((s - m) * SCALE)
            l = jnp.sum(e, axis=-1, keepdims=True)
            o = _mm_n(e.astype(jnp.bfloat16), lambda k, n: vb[g, n * T:(n + 1) * T, k * T:(k + 1) * T], W // T, GR // T)
            o = jnp.where(blk, o / l, 0.0).astype(jnp.bfloat16)
            r0 = pl.multiple_of(g * GR, GR)
            wog = wo.at[pl.ds(r0, GR)]
            return acc + _mm(o, lambda k, n: wog[k * T:(k + 1) * T, n * T:(n + 1) * T], GR // T, D // T)

        acc = lax.fori_loop(0, NG, group, jnp.zeros((M, D), jnp.float32))
        x = x + jnp.sum(acc, axis=0, keepdims=True)
        x1 = _ln(x)
        h = _ln(x1).astype(jnp.bfloat16)

        @pl.when(first)
        def _():
            w3_cp.wait()
        h = _gelu(_mm(h, lambda k, n: w3[k * T:(k + 1) * T, n * T:(n + 1) * T], D // T, F // T)).astype(jnp.bfloat16)

        @pl.when(first)
        def _():
            w4_cp.wait()
        return x + x1 + _mm(h, lambda k, n: w4[k * T:(k + 1) * T, n * T:(n + 1) * T], F // T, D // T)

    x = lax.fori_loop(0, 2, one_pass, x0)
    o_ref[0] = x[0:1, :].astype(o_ref.dtype)


@jax.jit
def pallas_interleave_layers__sliding_block_cached__mixer_s_mlp__decode_kernel(
    A_x, A_k_cache, A_v_cache, A_wq, A_wo, B_x, B_w1, B_w2, B_w3, B_w4,
):
    del B_x, B_w1, B_w2
    kt = jnp.swapaxes(A_k_cache, 2, 3).reshape(HD, SK)
    vt = jnp.swapaxes(A_v_cache, 2, 3).reshape(HD, SK)
    hbm = pl.BlockSpec(memory_space=pltpu.HBM)
    return pl.pallas_call(
        kernel,
        out_shape=jax.ShapeDtypeStruct((1, 1, D), jnp.bfloat16),
        in_specs=[pl.BlockSpec(memory_space=pltpu.VMEM)] + [hbm] * 6,
        out_specs=pl.BlockSpec(memory_space=pltpu.VMEM),
        scratch_shapes=[
            pltpu.VMEM((NG, GR, W), jnp.bfloat16),
            pltpu.VMEM((NG, GR, W), jnp.bfloat16),
            pltpu.VMEM((D, HD), jnp.bfloat16),
            pltpu.VMEM((HD, D), jnp.bfloat16),
            pltpu.VMEM((D, F), jnp.bfloat16),
            pltpu.VMEM((F, D), jnp.bfloat16),
            pltpu.VMEM((NG, M, GR), jnp.float32),
            pltpu.SemaphoreType.DMA((4 + 2 * NG,)),
        ],
        compiler_params=pltpu.CompilerParams(vmem_limit_bytes=126 * 1024 * 1024),
    )(A_x, kt, vt, A_wq, A_wo, B_w3, B_w4)
```

```python
import functools
import jax
import jax.numpy as jnp
import numpy as np
from jax import lax
import jax.experimental.pallas as pl
import jax.experimental.pallas.tpu as pltpu

H, DH, SK, W, D, F = 32, 192, 32768, 4096, 640, 1536
HD = H * DH
G = 4
NG = H // G
GR = G * DH
M = 8
T = 128
NC = 4
EPS = 1e-5
SCALE = DH ** -0.5
NA = int("4")
SB = int("2")
LINKX = [int(v) for v in "0".split(",")]
QOPQ = int("0")
BARRIER = int("1")
SCHED = "v4,q0,q1,q2;s0,s1,s2,s4,v5,q3,p0,p1;s3,s5,v6,p2,p3,p4;s6,v7,p5,p6;s7,p7"
ORDER = "0"
f32, bf16, u32 = jnp.float32, jnp.bfloat16, jnp.uint32


def _ln(x):
    m = jnp.mean(x, axis=-1, keepdims=True)
    xc = x - m
    v = jnp.mean(xc * xc, axis=-1, keepdims=True)
    return xc / jnp.sqrt(v + EPS)


def _gelu(x):
    c = np.float32(np.sqrt(2.0 / np.pi))
    return 0.5 * x * (1.0 + jnp.tanh(c * (x + 0.044715 * (x * x * x))))


def _dot(a, b):
    return jnp.dot(a, b, preferred_element_type=f32)


def _mm(a, tile, nk, nn):
    outs = [None] * nn
    for k in range(nk):
        ak = a[:, k * T:(k + 1) * T]
        for n in range(nn):
            d = _dot(ak, tile(k, n))
            outs[n] = d if outs[n] is None else outs[n] + d
    return outs


def _mm_n(a, tile, nk, nn):
    outs = []
    for n in range(nn):
        acc = None
        for k in range(nk):
            d = _dot(a[:, k * T:(k + 1) * T], tile(k, n))
            acc = d if acc is None else acc + d
        outs.append(acc)
    return outs


def _cat(xs):
    return jnp.concatenate(xs, axis=1)


def kernel(x_ref, k_hbm, v_hbm, wq_hbm, wo_hbm, w3_hbm, w4_hbm, o_ref,
           kb, vb, wq, wo, w3, w4, qc, ss, es, ls, qbs, os_, sems):
    KR = HD // NC
    VR = HD // 8 // NC

    def k_copy(g):
        return pltpu.make_async_copy(
            k_hbm.at[pl.ds(g * GR, GR), pl.ds(SK - W, W)], kb.at[pl.ds(g * GR, GR)], sems.at[NC + 4 + g])

    regions = [r.split(",") for r in SCHED.split(";")]
    kneed = []
    for items in regions:
        kneed.append([int(it[1:]) for it in items if it[0] in "vq"])

    def v_copy(c):
        return pltpu.make_async_copy(
            v_hbm.at[pl.ds(c * VR, VR), pl.ds((SK - W) // 16, W // 16)], vb.at[pl.ds(c * VR, VR)], sems.at[c])

    wq_cp = pltpu.make_async_copy(wq_hbm, wq, sems.at[NC])
    wo_cp = pltpu.make_async_copy(wo_hbm, wo, sems.at[NC + 1])
    w3_cp = pltpu.make_async_copy(w3_hbm, w3, sems.at[NC + 2])
    w4_cp = pltpu.make_async_copy(w4_hbm, w4, sems.at[NC + 3])
    for c in range(NC):
        v_copy(c).start()
    wq_cp.start()
    for gs in kneed:
        for g in gs:
            k_copy(g).start()
    wo_cp.start()
    w3_cp.start()
    w4_cp.start()

    row = lax.broadcasted_iota(jnp.int32, (M, GR), 0)
    col = lax.broadcasted_iota(jnp.int32, (M, GR), 1)
    blk = (col >= row * DH) & (col < row * DH + DH)
    vb32 = vb.bitcast(u32)
    ss[...] = jnp.zeros(ss.shape, f32)

    x0 = jnp.broadcast_to(x_ref[0].astype(f32), (M, D))

    def one_pass(p, x):
        first = p == 0
        never = jnp.full((M, T), p, jnp.int32) == 7

        @pl.when(first)
        def _():
            def chunk(c, carry):
                v_copy(c).wait()

                def tr(j, carry2):
                    r = pl.multiple_of(c * VR + j * 16, 16)
                    for a in range(W // 256):
                        xf = vb[pl.ds(r, 16), 16 * a:16 * a + 16, :].astype(f32)
                        ys = [xf[:, 8 * b:8 * b + 8, :].reshape(T, T).T.astype(bf16) for b in range(2)]
                        for b in range(2):
                            vb[pl.ds(r + 8 * b, 8), 16 * a:16 * a + 16, :] = ys[b].reshape(8, 16, T)
                    return carry2
                lax.fori_loop(0, VR // 16, tr, 0)
                return carry
            lax.fori_loop(0, NC, chunk, 0)
            wq_cp.wait()

        xn = _ln(x).astype(bf16)
        gorder = list(range(NA, NG)) + list(range(NA))
        qb = {}

        def qproj(g):
            q = _mm(xn, lambda k, n: wq[k * T:(k + 1) * T, g * GR + n * T:g * GR + (n + 1) * T], D // T, GR // T)
            if g < NA:
                qbs[g] = jnp.where(blk, _cat(q), 0.0).astype(bf16)
            else:
                for n in range(GR // T):
                    qq = q[n].astype(bf16).astype(f32)
                    r0 = (g - NA) * GR + n * T
                    qc[r0:r0 + T, :] = jnp.broadcast_to(qq[0:1, :], (T, T)).T

        def softmax(g):
            s = ss[g]
            m = jnp.max(s, axis=-1, keepdims=True)
            e = jnp.exp((s - m) * SCALE)
            l = jnp.sum(e, axis=-1, keepdims=True)
            es[g] = e.astype(bf16)
            ls[g] = jnp.broadcast_to(l, (M, T))

        NBK = 8

        def qk_mxu(g):
            for nb in range(W // T // NBK):
                outs = _mm(qbs.at[g], lambda k, n: kb[g * GR + k * T:g * GR + (k + 1) * T,
                                                   (nb * NBK + n) * T:(nb * NBK + n + 1) * T], GR // T, NBK)
                ss[g, :, nb * NBK * T:(nb + 1) * NBK * T] = _cat(outs)

        link = {"prev": None}

        def qk_vpu(g, hi):
            h = g * G + hi
            nx = LINKX[min(h - NA * G, len(LINKX) - 1)]
            for sb in range(W // T // SB):
                acc = [None] * SB
                zoff = pl.multiple_of((p >> 3) * (8 * (1 + (h * 64 + sb) % QOPQ)), 8) if QOPQ else 0
                for r in range(DH // 8):
                    if QOPQ:
                        qv = qc[pl.ds(zoff + (h * DH - NA * GR) + 8 * r, 8), :]
                    else:
                        qv = qc[(h * DH - NA * GR) + 8 * r:(h * DH - NA * GR) + 8 * r + 8, :]
                    kk = kb[h * DH + 8 * r:h * DH + 8 * r + 8, sb * SB * T:(sb + 1) * SB * T].astype(f32)
                    for t in range(SB):
                        xx = kk[:, t * T:(t + 1) * T] * qv
                        if r == 0:
                            acc[t] = xx if link["prev"] is None else jnp.where(never, link["prev"], xx)
                        else:
                            acc[t] = acc[t] + xx
                prev = None
                for t in range(SB):
                    a = acc[t]
                    if prev is not None and nx >= t:
                        a = jnp.where(never, prev, a)
                    red = jnp.sum(a, axis=0, keepdims=True)
                    n = sb * SB + t
                    ss[g, hi:hi + 1, n * T:(n + 1) * T] = red
                    prev = jnp.broadcast_to(red, (M, T))
                link["prev"] = prev

        def pv(g):
            def tile(k, n):
                J = g * (GR // T) + n
                a, b = k // 2, k % 2
                w = vb32[16 * J + 8 * b:16 * J + 8 * b + 8, 8 * a:8 * a + 8, :]
                return pltpu.bitcast(w.reshape(64, T), bf16)
            o = _cat(_mm_n(es.at[g], tile, W // T, GR // T))
            os_[:, g * GR:(g + 1) * GR] = jnp.where(blk, o / ls[g][:, 0:1], 0.0)

        one = (p >> 3) + 1

        def region(fn):
            if BARRIER:
                def body(i, c):
                    fn()
                    return c
                lax.fori_loop(0, one, body, 0)
            else:
                fn()

        def run(items):
            def fn():
                link["prev"] = None
                for it in items:
                    kind, g = it[0], int(it[1:])
                    if kind == "v":
                        for hi in range(G):
                            qk_vpu(g, hi)
                    elif kind == "q":
                        qk_mxu(g)
                    elif kind == "s":
                        softmax(g)
                    elif kind == "p":
                        pv(g)
            return fn

        def r0():
            for g in gorder:
                qproj(g)
        region(r0)
        for items, gs in zip(regions, kneed):
            if gs:
                @pl.when(first)
                def _():
                    for g in gs:
                        k_copy(g).wait()
            region(run(items))

        @pl.when(first)
        def _():
            wo_cp.wait()
        acc = _cat(_mm(os_[...].astype(bf16), lambda k, n: wo[k * T:(k + 1) * T, n * T:(n + 1) * T], HD // T, D // T))
        x = x + jnp.sum(acc, axis=0, keepdims=True)
        x1 = _ln(x)
        h = _ln(x1).astype(bf16)

        @pl.when(first)
        def _():
            w3_cp.wait()
        h = _gelu(_cat(_mm(h, lambda k, n: w3[k * T:(k + 1) * T, n * T:(n + 1) * T], D // T, F // T))).astype(bf16)

        @pl.when(first)
        def _():
            w4_cp.wait()
        return x + x1 + _cat(_mm(h, lambda k, n: w4[k * T:(k + 1) * T, n * T:(n + 1) * T], F // T, D // T))

    x = lax.fori_loop(0, 2, one_pass, x0)
    o_ref[0] = x[0:1, :].astype(o_ref.dtype)


@jax.jit
def pallas_interleave_layers__sliding_block_cached__mixer_s_mlp__decode_kernel(
    A_x, A_k_cache, A_v_cache, A_wq, A_wo, B_x, B_w1, B_w2, B_w3, B_w4,
):
    del B_x, B_w1, B_w2
    kt = jnp.swapaxes(A_k_cache, 2, 3).reshape(HD, SK)
    vt = jnp.swapaxes(A_v_cache, 2, 3).reshape(HD // 8, 8, SK // T, T).transpose(0, 2, 1, 3).reshape(HD // 8, SK // 16, T)
    hbm = pl.BlockSpec(memory_space=pltpu.HBM)
    return pl.pallas_call(
        kernel,
        out_shape=jax.ShapeDtypeStruct((1, 1, D), bf16),
        in_specs=[pl.BlockSpec(memory_space=pltpu.VMEM)] + [hbm] * 6,
        out_specs=pl.BlockSpec(memory_space=pltpu.VMEM),
        scratch_shapes=[
            pltpu.VMEM((HD, W), bf16),
            pltpu.VMEM((HD // 8, W // 16, T), bf16),
            pltpu.VMEM((D, HD), bf16),
            pltpu.VMEM((HD, D), bf16),
            pltpu.VMEM((D, F), bf16),
            pltpu.VMEM((F, D), bf16),
            pltpu.VMEM(((NG - NA) * GR, T), f32),
            pltpu.VMEM((NG, M, W), f32),
            pltpu.VMEM((NG, M, W), bf16),
            pltpu.VMEM((NG, M, T), f32),
            pltpu.VMEM((NA, M, GR), bf16),
            pltpu.VMEM((M, HD), f32),
            pltpu.SemaphoreType.DMA((NC + 4 + NG,)),
        ],
        compiler_params=pltpu.CompilerParams(vmem_limit_bytes=126 * 1024 * 1024),
    )(A_x, kt, vt, A_wq, A_wo, B_w3, B_w4)
```

```python
import functools
import jax
import jax.numpy as jnp
import numpy as np
from jax import lax
import jax.experimental.pallas as pl
import jax.experimental.pallas.tpu as pltpu

H, DH, SK, W, D, F = 32, 192, 32768, 4096, 640, 1536
HD = H * DH
GS = [int(v) for v in "4,4,4,2,4,4,4,4,2".split(",")]
assert sum(GS) == H
NG = len(GS)
GH = [sum(GS[:i]) for i in range(NG)]
GMAX = max(GS)
LN2 = int("1")
LMODE = int("0")
N1 = int("24")
M = 8
T = 128
NC = 4
EPS = 1e-5
SCALE = DH ** -0.5
NA = int("4")
SB = int("2")
LINKX = [int(v) for v in "0".split(",")]
QOPQ = int("0")
BARRIER = int("1")
SCHED = "j4,j5,j6,j7,j8,j0,j1,j2,j3;v4,q0,q1,q3;s0,s1,s3,s4,v5,q2,p0,p3;s2,s5,v6,p1,p2,p4.0;s6,v7,p4.1,p5,p6;s7,v8,p7;s8,p8"
ORDER = "0"
f32, bf16, u32 = jnp.float32, jnp.bfloat16, jnp.uint32


def _ln(x):
    m = jnp.mean(x, axis=-1, keepdims=True)
    xc = x - m
    v = jnp.mean(xc * xc, axis=-1, keepdims=True)
    return xc * lax.rsqrt(v + EPS)


def _ln2(x):
    m = jnp.mean(x, axis=-1, keepdims=True)
    xc = x - m
    v = jnp.mean(xc * xc, axis=-1, keepdims=True)
    r = lax.rsqrt(v + EPS)
    x1 = xc * r
    return x1, x1 * lax.rsqrt(v * r * r + EPS)


def _gelu(x):
    c = np.float32(np.sqrt(2.0 / np.pi))
    return 0.5 * x * (1.0 + jnp.tanh(c * (x + 0.044715 * (x * x * x))))


def _dot(a, b):
    return jnp.dot(a, b, preferred_element_type=f32)


def _mm(a, tile, nk, nn):
    outs = [None] * nn
    for k in range(nk):
        ak = a[:, k * T:(k + 1) * T]
        for n in range(nn):
            d = _dot(ak, tile(k, n))
            outs[n] = d if outs[n] is None else outs[n] + d
    return outs


def _mm_n(a, tile, nk, nn):
    outs = []
    for n in range(nn):
        acc = None
        for k in range(nk):
            d = _dot(a[:, k * T:(k + 1) * T], tile(k, n))
            acc = d if acc is None else acc + d
        outs.append(acc)
    return outs


def _cat(xs):
    return jnp.concatenate(xs, axis=1)


def kernel(x_ref, k_hbm, v_hbm, wq_hbm, wo_hbm, w3_hbm, w4_hbm, o_ref,
           kb, vb, wq, wo, w3, w4, qc, ss, es, ls, qbs, os_, sems):
    VR = HD // 8 // NC

    def k_copy(g):
        return pltpu.make_async_copy(
            k_hbm.at[pl.ds(GH[g] * DH, GS[g] * DH), pl.ds(SK - W, W)], kb.at[pl.ds(GH[g] * DH, GS[g] * DH)],
            sems.at[NC + 4 + g])

    regions = [r.split(",") for r in SCHED.split(";")]
    kneed = []
    for items in regions:
        gs = []
        for it in items:
            if it[0] in "vq":
                g = int(it[1:].split(".")[0])
                if not any(g in x for x in kneed) and g not in gs:
                    gs.append(g)
        kneed.append(gs)

    def v_copy(c):
        return pltpu.make_async_copy(
            v_hbm.at[pl.ds(c * VR, VR), pl.ds((SK - W) // 16, W // 16)], vb.at[pl.ds(c * VR, VR)], sems.at[c])

    wq_cp = pltpu.make_async_copy(wq_hbm, wq, sems.at[NC])
    wo_cp = pltpu.make_async_copy(wo_hbm, wo, sems.at[NC + 1])
    w3_cp = pltpu.make_async_copy(w3_hbm, w3, sems.at[NC + 2])
    w4_cp = pltpu.make_async_copy(w4_hbm, w4, sems.at[NC + 3])
    for c in range(NC):
        v_copy(c).start()
    wq_cp.start()
    for gs in kneed:
        for g in gs:
            k_copy(g).start()
    wo_cp.start()
    w3_cp.start()
    w4_cp.start()

    def blk(n):
        row = lax.broadcasted_iota(jnp.int32, (M, n * DH), 0)
        col = lax.broadcasted_iota(jnp.int32, (M, n * DH), 1)
        return (col >= row * DH) & (col < row * DH + DH)
    HB = GH[NA]
    vb32 = vb.bitcast(u32)
    ss[...] = jnp.zeros(ss.shape, f32)

    x0 = jnp.broadcast_to(x_ref[0].astype(f32), (M, D))

    def one_pass(p, x):
        first = p == 0
        never = jnp.full((M, T), p, jnp.int32) == 7

        @pl.when(first)
        def _():
            def chunk(c, carry):
                v_copy(c).wait()

                def tr(j, carry2):
                    r = pl.multiple_of(c * VR + j * 16, 16)
                    for a in range(W // 256):
                        xf = vb[pl.ds(r, 16), 16 * a:16 * a + 16, :].astype(f32)
                        ys = [xf[:, 8 * b:8 * b + 8, :].reshape(T, T).T.astype(bf16) for b in range(2)]
                        for b in range(2):
                            vb[pl.ds(r + 8 * b, 8), 16 * a:16 * a + 16, :] = ys[b].reshape(8, 16, T)
                    return carry2
                lax.fori_loop(0, VR // 16, tr, 0)
                return carry
            lax.fori_loop(0, NC, chunk, 0)
            wq_cp.wait()

        xn = _ln(x).astype(bf16)
        gorder = list(range(NA, NG)) + list(range(NA))
        qb = {}

        def qproj(g):
            r0, nt = GH[g] * DH, GS[g] * DH // T
            q = _mm(xn, lambda k, n: wq[k * T:(k + 1) * T, r0 + n * T:r0 + (n + 1) * T], D // T, nt)
            if g < NA:
                qbs[:, r0:r0 + nt * T] = jnp.where(blk(GS[g]), _cat(q), 0.0).astype(bf16)
            else:
                for n in range(nt):
                    qq = q[n].astype(bf16).astype(f32)
                    c0 = r0 - HB * DH + n * T
                    qc[c0:c0 + T, :] = jnp.broadcast_to(qq[0:1, :], (T, T)).T

        def softmax(g):
            s = ss[g]
            m = jnp.max(s, axis=-1, keepdims=True)
            e = jnp.exp((s - m) * SCALE)
            l = jnp.sum(e, axis=-1, keepdims=True)
            es[g] = e.astype(bf16)
            ls[g] = jnp.broadcast_to(l, (M, T))

        NBK = 8

        def qk_mxu(g, part=None):
            r0, nt = GH[g] * DH, GS[g] * DH // T
            nbs = range(W // T // NBK)
            if part is not None:
                nbs = nbs[2 * part:2 * part + 2]
            for nb in nbs:
                outs = _mm(qbs.at[:, r0:r0 + nt * T],
                           lambda k, n: kb[r0 + k * T:r0 + (k + 1) * T, (nb * NBK + n) * T:(nb * NBK + n + 1) * T],
                           nt, NBK)
                ss[g, :, nb * NBK * T:(nb + 1) * NBK * T] = _cat(outs)

        link = {"prev": None}

        def qk_vpu(g, hi):
            h = GH[g] + hi
            for sb in range(W // T // SB):
                acc = [None] * SB
                acc2 = [None] * SB
                for r in range(DH // 8):
                    c0 = (h - HB) * DH + 8 * r
                    qv = qc[c0:c0 + 8, :]
                    kk = kb[h * DH + 8 * r:h * DH + 8 * r + 8, sb * SB * T:(sb + 1) * SB * T].astype(f32)
                    for t in range(SB):
                        xx = kk[:, t * T:(t + 1) * T] * qv
                        if r == 0:
                            acc[t] = xx if link["prev"] is None else jnp.where(never, link["prev"], xx)
                        elif r < N1:
                            acc[t] = acc[t] + xx
                        elif r == N1:
                            acc2[t] = xx
                        else:
                            acc2[t] = acc2[t] + xx
                for t in range(SB):
                    a = acc[t] if acc2[t] is None else acc[t] + acc2[t]
                    red = jnp.sum(a, axis=0, keepdims=True)
                    n = sb * SB + t
                    ss[g, hi:hi + 1, n * T:(n + 1) * T] = red
                if LMODE == 0:
                    link["prev"] = jnp.broadcast_to(red, (M, T))
                else:
                    link["prev"] = acc[SB - 1] if link.get("red") is None else jnp.where(never, link["red"], acc[SB - 1])
                    link["red"] = jnp.broadcast_to(red, (M, T))

        def pv(g, part=None):
            r0, nt = GH[g] * DH, GS[g] * DH // T
            ns = list(range(nt))
            if part is not None:
                ns = ns[3 * part:3 * part + 3]

            def tile(k, n):
                J = r0 // T + ns[n]
                a, b = k // 2, k % 2
                w = vb32[16 * J + 8 * b:16 * J + 8 * b + 8, 8 * a:8 * a + 8, :]
                return pltpu.bitcast(w.reshape(64, T), bf16)
            o = _mm_n(es.at[g], tile, W // T, len(ns))
            inv = 1.0 / ls[g]
            bm = blk(GS[g])
            for i, n in enumerate(ns):
                os_[:, r0 + n * T:r0 + (n + 1) * T] = jnp.where(bm[:, n * T:(n + 1) * T], o[i] * inv, 0.0)

        one = (p >> 3) + 1

        def region(fn):
            if BARRIER:
                def body(i, c):
                    fn()
                    return c
                lax.fori_loop(0, one, body, 0)
            else:
                fn()

        def run(items):
            def fn():
                link["prev"] = None
                link["red"] = None
                for it in items:
                    kind = it[0]
                    f = [int(v) for v in it[1:].split(".")]
                    g = f[0]
                    if kind == "v":
                        for hi in (range(GS[g]) if len(f) == 1 else f[1:]):
                            qk_vpu(g, hi)
                    elif kind == "q":
                        qk_mxu(*f)
                    elif kind == "s":
                        softmax(g)
                    elif kind == "p":
                        pv(*f)
                    elif kind == "j":
                        qproj(g)
            return fn

        for items, gs in zip(regions, kneed):
            if gs:
                @pl.when(first)
                def _():
                    for g in gs:
                        k_copy(g).wait()
            region(run(items))

        @pl.when(first)
        def _():
            wo_cp.wait()
        acc = _cat(_mm(os_[...].astype(bf16), lambda k, n: wo[k * T:(k + 1) * T, n * T:(n + 1) * T], HD // T, D // T))
        x = x + jnp.sum(acc, axis=0, keepdims=True)
        if LN2:
            x1, h = _ln2(x)
            h = h.astype(bf16)
        else:
            x1 = _ln(x)
            h = _ln(x1).astype(bf16)

        @pl.when(first)
        def _():
            w3_cp.wait()
        h = _gelu(_cat(_mm(h, lambda k, n: w3[k * T:(k + 1) * T, n * T:(n + 1) * T], D // T, F // T))).astype(bf16)

        @pl.when(first)
        def _():
            w4_cp.wait()
        return x + x1 + _cat(_mm(h, lambda k, n: w4[k * T:(k + 1) * T, n * T:(n + 1) * T], F // T, D // T))

    x = lax.fori_loop(0, 2, one_pass, x0)
    o_ref[0] = x[0:1, :].astype(o_ref.dtype)


@jax.jit
def pallas_interleave_layers__sliding_block_cached__mixer_s_mlp__decode_kernel(
    A_x, A_k_cache, A_v_cache, A_wq, A_wo, B_x, B_w1, B_w2, B_w3, B_w4,
):
    del B_x, B_w1, B_w2
    kt = jnp.swapaxes(A_k_cache, 2, 3).reshape(HD, SK)
    vt = jnp.swapaxes(A_v_cache, 2, 3).reshape(HD // 8, 8, SK // T, T).transpose(0, 2, 1, 3).reshape(HD // 8, SK // 16, T)
    hbm = pl.BlockSpec(memory_space=pltpu.HBM)
    return pl.pallas_call(
        kernel,
        out_shape=jax.ShapeDtypeStruct((1, 1, D), bf16),
        in_specs=[pl.BlockSpec(memory_space=pltpu.VMEM)] + [hbm] * 6,
        out_specs=pl.BlockSpec(memory_space=pltpu.VMEM),
        scratch_shapes=[
            pltpu.VMEM((HD, W), bf16),
            pltpu.VMEM((HD // 8, W // 16, T), bf16),
            pltpu.VMEM((D, HD), bf16),
            pltpu.VMEM((HD, D), bf16),
            pltpu.VMEM((D, F), bf16),
            pltpu.VMEM((F, D), bf16),
            pltpu.VMEM(((H - GH[NA]) * DH, T), f32),
            pltpu.VMEM((NG, M, W), f32),
            pltpu.VMEM((NG, M, W), bf16),
            pltpu.VMEM((NG, M, T), f32),
            pltpu.VMEM((M, GH[NA] * DH), bf16),
            pltpu.VMEM((M, HD), f32),
            pltpu.SemaphoreType.DMA((NC + 4 + NG,)),
        ],
        compiler_params=pltpu.CompilerParams(vmem_limit_bytes=126 * 1024 * 1024),
    )(A_x, kt, vt, A_wq, A_wo, B_w3, B_w4)
```

```python
import functools
import jax
import jax.numpy as jnp
import numpy as np
from jax import lax
import jax.experimental.pallas as pl
import jax.experimental.pallas.tpu as pltpu

H, DH, SK, W, D, F = 32, 192, 32768, 4096, 640, 1536
HD = H * DH
GS = [int(v) for v in "4,4,4,2,4,4,4,4,2".split(",")]
assert sum(GS) == H
NG = len(GS)
GH = [sum(GS[:i]) for i in range(NG)]
GMAX = max(GS)
LN2 = int("1")
LMODE = int("0")
N1 = int("24")
M = 8
T = 128
NC = 4
EPS = 1e-5
SCALE = DH ** -0.5
NA = int("4")
SB = int("2")
LINKX = [int(v) for v in "0".split(",")]
QOPQ = int("0")
BARRIER = int("1")
SCHED = "j4,j5,j6,j7,j8,j0,j1,j2,j3;v4,q0,q1,q3;s0,s1,s3,s4,v5,q2,p0,p3;s2,s5,v6,p1,p2,p4.0;s6,v7,p4.1,p5,p6;s7,v8,p7;s8,p8"
ORDER = "0"
f32, bf16, u32 = jnp.float32, jnp.bfloat16, jnp.uint32


def _ln(x):
    m = jnp.mean(x, axis=-1, keepdims=True)
    xc = x - m
    v = jnp.mean(xc * xc, axis=-1, keepdims=True)
    return xc * lax.rsqrt(v + EPS)


def _ln2(x):
    m = jnp.mean(x, axis=-1, keepdims=True)
    xc = x - m
    v = jnp.mean(xc * xc, axis=-1, keepdims=True)
    r = lax.rsqrt(v + EPS)
    x1 = xc * r
    return x1, x1 * lax.rsqrt(v * r * r + EPS)


def _gelu(x):
    c = np.float32(np.sqrt(2.0 / np.pi))
    return 0.5 * x * (1.0 + jnp.tanh(c * (x + 0.044715 * (x * x * x))))


def _dot(a, b):
    return jnp.dot(a, b, preferred_element_type=f32)


def _mm(a, tile, nk, nn):
    outs = [None] * nn
    for k in range(nk):
        ak = a[:, k * T:(k + 1) * T]
        for n in range(nn):
            d = _dot(ak, tile(k, n))
            outs[n] = d if outs[n] is None else outs[n] + d
    return outs


def _mm_n(a, tile, nk, nn):
    outs = []
    for n in range(nn):
        acc = None
        for k in range(nk):
            d = _dot(a[:, k * T:(k + 1) * T], tile(k, n))
            acc = d if acc is None else acc + d
        outs.append(acc)
    return outs


def _cat(xs):
    return jnp.concatenate(xs, axis=1)


def kernel(x_hbm, k_hbm, v_hbm, wq_hbm, wo_hbm, w3_hbm, w4_hbm, o_ref,
           kb, vb, wq, wo, w3, w4, qc, ss, es, ls, qbs, os_, x_ref, sems):
    VR = HD // 8 // NC

    def k_copy(g):
        return pltpu.make_async_copy(
            k_hbm.at[pl.ds(GH[g] * DH, GS[g] * DH), pl.ds(SK - W, W)], kb.at[pl.ds(GH[g] * DH, GS[g] * DH)],
            sems.at[NC + 4 + g])

    regions = [r.split(",") for r in SCHED.split(";")]
    kneed = []
    for items in regions:
        gs = []
        for it in items:
            if it[0] in "vq":
                g = int(it[1:].split(".")[0])
                if not any(g in x for x in kneed) and g not in gs:
                    gs.append(g)
        kneed.append(gs)

    def v_copy(c):
        return pltpu.make_async_copy(
            v_hbm.at[pl.ds(c * VR, VR), pl.ds((SK - W) // 16, W // 16)], vb.at[pl.ds(c * VR, VR)], sems.at[c])

    wq_cp = pltpu.make_async_copy(wq_hbm, wq, sems.at[NC])
    wo_cp = pltpu.make_async_copy(wo_hbm, wo, sems.at[NC + 1])
    w3_cp = pltpu.make_async_copy(w3_hbm, w3, sems.at[NC + 2])
    w4_cp = pltpu.make_async_copy(w4_hbm, w4, sems.at[NC + 3])
    x_cp = pltpu.make_async_copy(x_hbm, x_ref, sems.at[NC + 4 + NG])
    x_cp.start()
    for c in range(NC):
        v_copy(c).start()
    wq_cp.start()
    for gs in kneed:
        for g in gs:
            k_copy(g).start()
    wo_cp.start()
    w3_cp.start()
    w4_cp.start()

    def blk(n):
        row = lax.broadcasted_iota(jnp.int32, (M, n * DH), 0)
        col = lax.broadcasted_iota(jnp.int32, (M, n * DH), 1)
        return (col >= row * DH) & (col < row * DH + DH)
    HB = GH[NA]
    vb32 = vb.bitcast(u32)
    ss[...] = jnp.zeros(ss.shape, f32)

    x_cp.wait()
    x0 = jnp.broadcast_to(x_ref[0].astype(f32), (M, D))

    def one_pass(p, x):
        first = p == 0
        never = jnp.full((M, T), p, jnp.int32) == 7

        @pl.when(first)
        def _():
            def chunk(c, carry):
                v_copy(c).wait()

                def tr(j, carry2):
                    r = pl.multiple_of(c * VR + j * 16, 16)
                    for a in range(W // 256):
                        xf = vb[pl.ds(r, 16), 16 * a:16 * a + 16, :].astype(f32)
                        ys = [xf[:, 8 * b:8 * b + 8, :].reshape(T, T).T.astype(bf16) for b in range(2)]
                        for b in range(2):
                            vb[pl.ds(r + 8 * b, 8), 16 * a:16 * a + 16, :] = ys[b].reshape(8, 16, T)
                    return carry2
                lax.fori_loop(0, VR // 16, tr, 0)
                return carry
            lax.fori_loop(0, NC, chunk, 0)
            wq_cp.wait()

        xn = _ln(x).astype(bf16)
        gorder = list(range(NA, NG)) + list(range(NA))
        qb = {}

        def qproj(g):
            r0, nt = GH[g] * DH, GS[g] * DH // T
            q = _mm(xn, lambda k, n: wq[k * T:(k + 1) * T, r0 + n * T:r0 + (n + 1) * T], D // T, nt)
            if g < NA:
                qbs[:, r0:r0 + nt * T] = jnp.where(blk(GS[g]), _cat(q), 0.0).astype(bf16)
            else:
                for n in range(nt):
                    qq = q[n].astype(bf16).astype(f32)
                    c0 = r0 - HB * DH + n * T
                    qc[c0:c0 + T, :] = jnp.broadcast_to(qq[0:1, :], (T, T)).T

        def softmax(g):
            s = ss[g]
            m = jnp.max(s, axis=-1, keepdims=True)
            e = jnp.exp((s - m) * SCALE)
            l = jnp.sum(e, axis=-1, keepdims=True)
            es[g] = e.astype(bf16)
            ls[g] = jnp.broadcast_to(l, (M, T))

        NBK = 8

        def qk_mxu(g, part=None):
            r0, nt = GH[g] * DH, GS[g] * DH // T
            nbs = range(W // T // NBK)
            if part is not None:
                nbs = nbs[2 * part:2 * part + 2]
            for nb in nbs:
                outs = _mm(qbs.at[:, r0:r0 + nt * T],
                           lambda k, n: kb[r0 + k * T:r0 + (k + 1) * T, (nb * NBK + n) * T:(nb * NBK + n + 1) * T],
                           nt, NBK)
                ss[g, :, nb * NBK * T:(nb + 1) * NBK * T] = _cat(outs)

        link = {"prev": None}

        def qk_vpu(g, hi):
            h = GH[g] + hi
            for sb in range(W // T // SB):
                acc = [None] * SB
                acc2 = [None] * SB
                for r in range(DH // 8):
                    c0 = (h - HB) * DH + 8 * r
                    qv = qc[c0:c0 + 8, :]
                    kk = kb[h * DH + 8 * r:h * DH + 8 * r + 8, sb * SB * T:(sb + 1) * SB * T].astype(f32)
                    for t in range(SB):
                        xx = kk[:, t * T:(t + 1) * T] * qv
                        if r == 0:
                            acc[t] = xx if link["prev"] is None else jnp.where(never, link["prev"], xx)
                        elif r < N1:
                            acc[t] = acc[t] + xx
                        elif r == N1:
                            acc2[t] = xx
                        else:
                            acc2[t] = acc2[t] + xx
                for t in range(SB):
                    a = acc[t] if acc2[t] is None else acc[t] + acc2[t]
                    red = jnp.sum(a, axis=0, keepdims=True)
                    n = sb * SB + t
                    ss[g, hi:hi + 1, n * T:(n + 1) * T] = red
                if LMODE == 0:
                    link["prev"] = jnp.broadcast_to(red, (M, T))
                else:
                    link["prev"] = acc[SB - 1] if link.get("red") is None else jnp.where(never, link["red"], acc[SB - 1])
                    link["red"] = jnp.broadcast_to(red, (M, T))

        def pv(g, part=None):
            r0, nt = GH[g] * DH, GS[g] * DH // T
            ns = list(range(nt))
            if part is not None:
                ns = ns[3 * part:3 * part + 3]

            def tile(k, n):
                J = r0 // T + ns[n]
                a, b = k // 2, k % 2
                w = vb32[16 * J + 8 * b:16 * J + 8 * b + 8, 8 * a:8 * a + 8, :]
                return pltpu.bitcast(w.reshape(64, T), bf16)
            o = _mm_n(es.at[g], tile, W // T, len(ns))
            inv = 1.0 / ls[g]
            bm = blk(GS[g])
            for i, n in enumerate(ns):
                os_[:, r0 + n * T:r0 + (n + 1) * T] = jnp.where(bm[:, n * T:(n + 1) * T], o[i] * inv, 0.0)

        one = (p >> 3) + 1

        def region(fn):
            if BARRIER:
                def body(i, c):
                    fn()
                    return c
                lax.fori_loop(0, one, body, 0)
            else:
                fn()

        def run(items):
            def fn():
                link["prev"] = None
                link["red"] = None
                for it in items:
                    kind = it[0]
                    f = [int(v) for v in it[1:].split(".")]
                    g = f[0]
                    if kind == "v":
                        for hi in (range(GS[g]) if len(f) == 1 else f[1:]):
                            qk_vpu(g, hi)
                    elif kind == "q":
                        qk_mxu(*f)
                    elif kind == "s":
                        softmax(g)
                    elif kind == "p":
                        pv(*f)
                    elif kind == "j":
                        qproj(g)
            return fn

        for items, gs in zip(regions, kneed):
            if gs:
                @pl.when(first)
                def _():
                    for g in gs:
                        k_copy(g).wait()
            region(run(items))

        @pl.when(first)
        def _():
            wo_cp.wait()
        acc = _cat(_mm(os_[...].astype(bf16), lambda k, n: wo[k * T:(k + 1) * T, n * T:(n + 1) * T], HD // T, D // T))
        x = x + jnp.sum(acc, axis=0, keepdims=True)
        if LN2:
            x1, h = _ln2(x)
            h = h.astype(bf16)
        else:
            x1 = _ln(x)
            h = _ln(x1).astype(bf16)

        @pl.when(first)
        def _():
            w3_cp.wait()
        h = _gelu(_cat(_mm(h, lambda k, n: w3[k * T:(k + 1) * T, n * T:(n + 1) * T], D // T, F // T))).astype(bf16)

        @pl.when(first)
        def _():
            w4_cp.wait()
        return x + x1 + _cat(_mm(h, lambda k, n: w4[k * T:(k + 1) * T, n * T:(n + 1) * T], F // T, D // T))

    x = lax.fori_loop(0, 2, one_pass, x0)
    o_ref[0] = x[0:1, :].astype(o_ref.dtype)


@jax.jit
def pallas_interleave_layers__sliding_block_cached__mixer_s_mlp__decode_kernel(
    A_x, A_k_cache, A_v_cache, A_wq, A_wo, B_x, B_w1, B_w2, B_w3, B_w4,
):
    del B_x, B_w1, B_w2
    kt = jnp.swapaxes(A_k_cache, 2, 3).reshape(HD, SK)
    vt = jnp.swapaxes(A_v_cache, 2, 3).reshape(HD // 8, 8, SK // T, T).transpose(0, 2, 1, 3).reshape(HD // 8, SK // 16, T)
    hbm = pl.BlockSpec(memory_space=pltpu.HBM)
    return pl.pallas_call(
        kernel,
        out_shape=jax.ShapeDtypeStruct((1, 1, D), bf16),
        in_specs=[hbm] * 7,
        out_specs=pl.BlockSpec(memory_space=pltpu.VMEM),
        scratch_shapes=[
            pltpu.VMEM((HD, W), bf16),
            pltpu.VMEM((HD // 8, W // 16, T), bf16),
            pltpu.VMEM((D, HD), bf16),
            pltpu.VMEM((HD, D), bf16),
            pltpu.VMEM((D, F), bf16),
            pltpu.VMEM((F, D), bf16),
            pltpu.VMEM(((H - GH[NA]) * DH, T), f32),
            pltpu.VMEM((NG, M, W), f32),
            pltpu.VMEM((NG, M, W), bf16),
            pltpu.VMEM((NG, M, T), f32),
            pltpu.VMEM((M, GH[NA] * DH), bf16),
            pltpu.VMEM((M, HD), f32),
            pltpu.VMEM((1, 1, D), bf16),
            pltpu.SemaphoreType.DMA((NC + 5 + NG,)),
        ],
        compiler_params=pltpu.CompilerParams(vmem_limit_bytes=126 * 1024 * 1024),
    )(A_x, kt, vt, A_wq, A_wo, B_w3, B_w4)
```

```python
import functools
import jax
import jax.numpy as jnp
import numpy as np
from jax import lax
import jax.experimental.pallas as pl
import jax.experimental.pallas.tpu as pltpu

H, DH, SK, W, D, F = 32, 192, 32768, 4096, 640, 1536
HD = H * DH
GS = [int(v) for v in "4,4,4,4,4,4,4,4".split(",")]
assert sum(GS) == H
NG = len(GS)
GH = [sum(GS[:i]) for i in range(NG)]
GMAX = max(GS)
LN2 = int("1")
LMODE = int("0")
N1 = int("17")
M = 8
T = 128
NC = 4
EPS = 1e-5
SCALE = DH ** -0.5
NA = int("3")
SB = int("2")
LINKX = [int(v) for v in "0".split(",")]
QOPQ = int("0")
BARRIER = int("1")
SCHED = "j3,j4,j5,j6,j7,j0,j1,j2;v3,q0,q1;s0,s1,s3,v4,q2,p0;s2,s4,v5,p1,p2;s5,v6,p3,p4;s6,v7,p5,p6;s7,p7"
ORDER = "0"
f32, bf16, u32 = jnp.float32, jnp.bfloat16, jnp.uint32


def _ln(x):
    m = jnp.mean(x, axis=-1, keepdims=True)
    xc = x - m
    v = jnp.mean(xc * xc, axis=-1, keepdims=True)
    return xc * lax.rsqrt(v + EPS)


def _ln2(x):
    m = jnp.mean(x, axis=-1, keepdims=True)
    xc = x - m
    v = jnp.mean(xc * xc, axis=-1, keepdims=True)
    r = lax.rsqrt(v + EPS)
    x1 = xc * r
    return x1, x1 * lax.rsqrt(v * r * r + EPS)


def _gelu(x):
    c = np.float32(np.sqrt(2.0 / np.pi))
    return 0.5 * x * (1.0 + jnp.tanh(c * (x + 0.044715 * (x * x * x))))


def _dot(a, b):
    return jnp.dot(a, b, preferred_element_type=f32)


def _mm(a, tile, nk, nn):
    outs = [None] * nn
    for k in range(nk):
        ak = a[:, k * T:(k + 1) * T]
        for n in range(nn):
            d = _dot(ak, tile(k, n))
            outs[n] = d if outs[n] is None else outs[n] + d
    return outs


def _mm_n(a, tile, nk, nn):
    outs = []
    for n in range(nn):
        acc = None
        for k in range(nk):
            d = _dot(a[:, k * T:(k + 1) * T], tile(k, n))
            acc = d if acc is None else acc + d
        outs.append(acc)
    return outs


def _cat(xs):
    return jnp.concatenate(xs, axis=1)


def kernel(x_hbm, k_hbm, v_hbm, wq_hbm, wo_hbm, w3_hbm, w4_hbm, o_ref,
           kb, vb, wq, wo, w3, w4, qc, ss, es, ls, qbs, os_, x_ref, sems):
    VR = HD // 8 // NC

    def k_copy(g):
        return pltpu.make_async_copy(
            k_hbm.at[pl.ds(GH[g] * DH // 8, GS[g] * DH // 8), pl.ds((SK - W) // 16, W // 16)],
            kb.at[pl.ds(GH[g] * DH // 8, GS[g] * DH // 8)], sems.at[NC + 4 + g])

    regions = [r.split(",") for r in SCHED.split(";")]
    kneed = []
    for items in regions:
        gs = []
        for it in items:
            if it[0] in "vq":
                g = int(it[1:].split(".")[0])
                if not any(g in x for x in kneed) and g not in gs:
                    gs.append(g)
        kneed.append(gs)

    def v_copy(c):
        return pltpu.make_async_copy(
            v_hbm.at[pl.ds(c * VR, VR), pl.ds((SK - W) // 16, W // 16)], vb.at[pl.ds(c * VR, VR)], sems.at[c])

    wq_cp = pltpu.make_async_copy(wq_hbm, wq, sems.at[NC])
    wo_cp = pltpu.make_async_copy(wo_hbm, wo, sems.at[NC + 1])
    w3_cp = pltpu.make_async_copy(w3_hbm, w3, sems.at[NC + 2])
    w4_cp = pltpu.make_async_copy(w4_hbm, w4, sems.at[NC + 3])
    x_cp = pltpu.make_async_copy(x_hbm, x_ref, sems.at[NC + 4 + NG])
    x_cp.start()
    for c in range(NC):
        v_copy(c).start()
    wq_cp.start()
    for gs in kneed:
        for g in gs:
            k_copy(g).start()
    wo_cp.start()
    w3_cp.start()
    w4_cp.start()

    def blk(n):
        row = lax.broadcasted_iota(jnp.int32, (M, n * DH), 0)
        col = lax.broadcasted_iota(jnp.int32, (M, n * DH), 1)
        return (col >= row * DH) & (col < row * DH + DH)
    HB = GH[NA]
    vb32 = vb.bitcast(u32)
    kb32 = kb.bitcast(u32)

    def k_retile(g):
        def body(j, c):
            r = pl.multiple_of(GH[g] * DH // 8 + j * 16, 8)
            for a in range(W // 256):
                xf = kb[pl.ds(r, 16), 16 * a:16 * a + 16, :].astype(f32)
                for b in range(2):
                    y = xf[:, 8 * b:8 * b + 8, :].reshape(8, 16, T).astype(bf16)
                    kb[pl.ds(r + 8 * b, 8), 16 * a:16 * a + 16, :] = y
            return c
        lax.fori_loop(0, GS[g] * DH // T, body, 0)
    ss[...] = jnp.zeros(ss.shape, f32)

    x_cp.wait()
    x0 = jnp.broadcast_to(x_ref[0].astype(f32), (M, D))

    def one_pass(p, x):
        first = p == 0
        never = jnp.full((M, T), p, jnp.int32) == 7

        @pl.when(first)
        def _():
            def chunk(c, carry):
                v_copy(c).wait()

                def tr(j, carry2):
                    r = pl.multiple_of(c * VR + j * 16, 16)
                    for a in range(W // 256):
                        xf = vb[pl.ds(r, 16), 16 * a:16 * a + 16, :].astype(f32)
                        ys = [xf[:, 8 * b:8 * b + 8, :].reshape(T, T).T.astype(bf16) for b in range(2)]
                        for b in range(2):
                            vb[pl.ds(r + 8 * b, 8), 16 * a:16 * a + 16, :] = ys[b].reshape(8, 16, T)
                    return carry2
                lax.fori_loop(0, VR // 16, tr, 0)
                return carry
            lax.fori_loop(0, NC, chunk, 0)
            wq_cp.wait()

        xn = _ln(x).astype(bf16)
        gorder = list(range(NA, NG)) + list(range(NA))
        qb = {}

        def qproj(g):
            r0, nt = GH[g] * DH, GS[g] * DH // T
            q = _mm(xn, lambda k, n: wq[k * T:(k + 1) * T, r0 + n * T:r0 + (n + 1) * T], D // T, nt)
            if g < NA:
                qbs[:, r0:r0 + nt * T] = jnp.where(blk(GS[g]), _cat(q), 0.0).astype(bf16)
            else:
                for n in range(nt):
                    qq = q[n].astype(bf16).astype(f32)
                    c0 = r0 - HB * DH + n * T
                    qc[c0:c0 + T, :] = jnp.broadcast_to(qq[0:1, :], (T, T)).T

        def softmax(g):
            s = ss[g]
            m = jnp.max(s, axis=-1, keepdims=True)
            e = jnp.exp((s - m) * SCALE)
            l = jnp.sum(e, axis=-1, keepdims=True)
            es[g] = e.astype(bf16)
            ls[g] = jnp.broadcast_to(l, (M, T))

        NBK = 8

        def ktile(i, n):
            a, b = n // 2, n % 2
            return pltpu.bitcast(kb32[i + 8 * b:i + 8 * b + 8, 8 * a:8 * a + 8, :].reshape(64, T), bf16)

        def qk_mxu(g, part=None):
            r0, nt = GH[g] * DH, GS[g] * DH // T
            nbs = range(W // T // NBK)
            if part is not None:
                nbs = nbs[2 * part:2 * part + 2]
            for nb in nbs:
                outs = _mm(qbs.at[:, r0:r0 + nt * T],
                           lambda k, n: ktile(r0 // 8 + 16 * k, nb * NBK + n), nt, NBK)
                ss[g, :, nb * NBK * T:(nb + 1) * NBK * T] = _cat(outs)

        link = {"prev": None}

        def qk_vpu(g, hi):
            h = GH[g] + hi
            for sb in range(W // T // SB):
                acc = [None] * SB
                acc2 = [None] * SB
                for r in range(DH // 8):
                    c0 = (h - HB) * DH + 8 * r
                    qv = qc[c0:c0 + 8, :]
                    kk = pltpu.bitcast(kb32[h * DH // 8 + r, 8 * sb:8 * sb + 8, :], bf16).astype(f32)
                    for t in range(SB):
                        xx = kk[8 * t:8 * t + 8, :] * qv
                        if r == 0:
                            acc[t] = xx if link["prev"] is None else jnp.where(never, link["prev"], xx)
                        elif r < N1:
                            acc[t] = acc[t] + xx
                        elif r == N1:
                            acc2[t] = xx
                        else:
                            acc2[t] = acc2[t] + xx
                for t in range(SB):
                    a = acc[t] if acc2[t] is None else acc[t] + acc2[t]
                    red = jnp.sum(a, axis=0, keepdims=True)
                    n = sb * SB + t
                    ss[g, hi:hi + 1, n * T:(n + 1) * T] = red
                if LMODE == 0:
                    link["prev"] = jnp.broadcast_to(red, (M, T))
                else:
                    link["prev"] = acc[SB - 1] if link.get("red") is None else jnp.where(never, link["red"], acc[SB - 1])
                    link["red"] = jnp.broadcast_to(red, (M, T))

        def pv(g, part=None):
            r0, nt = GH[g] * DH, GS[g] * DH // T
            ns = list(range(nt))
            if part is not None:
                ns = ns[3 * part:3 * part + 3]

            def tile(k, n):
                J = r0 // T + ns[n]
                a, b = k // 2, k % 2
                w = vb32[16 * J + 8 * b:16 * J + 8 * b + 8, 8 * a:8 * a + 8, :]
                return pltpu.bitcast(w.reshape(64, T), bf16)
            o = _mm_n(es.at[g], tile, W // T, len(ns))
            inv = 1.0 / ls[g]
            bm = blk(GS[g])
            for i, n in enumerate(ns):
                os_[:, r0 + n * T:r0 + (n + 1) * T] = jnp.where(bm[:, n * T:(n + 1) * T], o[i] * inv, 0.0)

        one = (p >> 3) + 1

        def region(fn):
            if BARRIER:
                def body(i, c):
                    fn()
                    return c
                lax.fori_loop(0, one, body, 0)
            else:
                fn()

        def run(items):
            def fn():
                link["prev"] = None
                link["red"] = None
                for it in items:
                    kind = it[0]
                    f = [int(v) for v in it[1:].split(".")]
                    g = f[0]
                    if kind == "v":
                        for hi in (range(GS[g]) if len(f) == 1 else f[1:]):
                            qk_vpu(g, hi)
                    elif kind == "q":
                        qk_mxu(*f)
                    elif kind == "s":
                        softmax(g)
                    elif kind == "p":
                        pv(*f)
                    elif kind == "j":
                        qproj(g)
            return fn

        for items, gs in zip(regions, kneed):
            if gs:
                @pl.when(first)
                def _():
                    for g in gs:
                        k_copy(g).wait()
                        if g < NA:
                            k_retile(g)
            region(run(items))

        @pl.when(first)
        def _():
            wo_cp.wait()
        acc = _cat(_mm(os_[...].astype(bf16), lambda k, n: wo[k * T:(k + 1) * T, n * T:(n + 1) * T], HD // T, D // T))
        x = x + jnp.sum(acc, axis=0, keepdims=True)
        if LN2:
            x1, h = _ln2(x)
            h = h.astype(bf16)
        else:
            x1 = _ln(x)
            h = _ln(x1).astype(bf16)

        @pl.when(first)
        def _():
            w3_cp.wait()
        h = _gelu(_cat(_mm(h, lambda k, n: w3[k * T:(k + 1) * T, n * T:(n + 1) * T], D // T, F // T))).astype(bf16)

        @pl.when(first)
        def _():
            w4_cp.wait()
        return x + x1 + _cat(_mm(h, lambda k, n: w4[k * T:(k + 1) * T, n * T:(n + 1) * T], F // T, D // T))

    x = lax.fori_loop(0, 2, one_pass, x0)
    o_ref[0] = x[0:1, :].astype(o_ref.dtype)


@jax.jit
def pallas_interleave_layers__sliding_block_cached__mixer_s_mlp__decode_kernel(
    A_x, A_k_cache, A_v_cache, A_wq, A_wo, B_x, B_w1, B_w2, B_w3, B_w4,
):
    del B_x, B_w1, B_w2
    kt = jnp.swapaxes(A_k_cache, 2, 3).reshape(HD // 8, 8, SK // T, T).transpose(0, 2, 1, 3).reshape(HD // 8, SK // 16, T)
    vt = jnp.swapaxes(A_v_cache, 2, 3).reshape(HD // 8, 8, SK // T, T).transpose(0, 2, 1, 3).reshape(HD // 8, SK // 16, T)
    hbm = pl.BlockSpec(memory_space=pltpu.HBM)
    return pl.pallas_call(
        kernel,
        out_shape=jax.ShapeDtypeStruct((1, 1, D), bf16),
        in_specs=[hbm] * 7,
        out_specs=pl.BlockSpec(memory_space=pltpu.VMEM),
        scratch_shapes=[
            pltpu.VMEM((HD // 8, W // 16, T), bf16),
            pltpu.VMEM((HD // 8, W // 16, T), bf16),
            pltpu.VMEM((D, HD), bf16),
            pltpu.VMEM((HD, D), bf16),
            pltpu.VMEM((D, F), bf16),
            pltpu.VMEM((F, D), bf16),
            pltpu.VMEM(((H - GH[NA]) * DH, T), f32),
            pltpu.VMEM((NG, M, W), f32),
            pltpu.VMEM((NG, M, W), bf16),
            pltpu.VMEM((NG, M, T), f32),
            pltpu.VMEM((M, GH[NA] * DH), bf16),
            pltpu.VMEM((M, HD), f32),
            pltpu.VMEM((1, 1, D), bf16),
            pltpu.SemaphoreType.DMA((NC + 5 + NG,)),
        ],
        compiler_params=pltpu.CompilerParams(vmem_limit_bytes=126 * 1024 * 1024),
    )(A_x, kt, vt, A_wq, A_wo, B_w3, B_w4)
```

```python
import functools
import jax
import jax.numpy as jnp
import numpy as np
from jax import lax
import jax.experimental.pallas as pl
import jax.experimental.pallas.tpu as pltpu

H, DH, SK, W, D, F = 32, 192, 32768, 4096, 640, 1536
HD = H * DH
GS = [int(v) for v in "4,4,4,4,4,4,4,4".split(",")]
assert sum(GS) == H
NG = len(GS)
GH = [sum(GS[:i]) for i in range(NG)]
GMAX = max(GS)
TAIL = int("1")
LN2 = int("1")
LMODE = int("0")
N1 = int("17")
M = 8
T = 128
NC = 4
EPS = 1e-5
SCALE = DH ** -0.5
NA = int("3")
SB = int("2")
LINKX = [int(v) for v in "0".split(",")]
QOPQ = int("0")
BARRIER = int("1")
SCHED = "j3,j4,j5,j6,j7,j0,j1,j2;v3,q0,q1;s0,s1,s3,v4,q2,p0;s2,s4,v5,p1,p2;s5,v6,p3,p4;s6,v7,p5,p6"
ORDER = "0"
f32, bf16, u32 = jnp.float32, jnp.bfloat16, jnp.uint32


def _ln(x):
    m = jnp.mean(x, axis=-1, keepdims=True)
    xc = x - m
    v = jnp.mean(xc * xc, axis=-1, keepdims=True)
    return xc * lax.rsqrt(v + EPS)


def _ln2(x):
    m = jnp.mean(x, axis=-1, keepdims=True)
    xc = x - m
    v = jnp.mean(xc * xc, axis=-1, keepdims=True)
    r = lax.rsqrt(v + EPS)
    x1 = xc * r
    return x1, x1 * lax.rsqrt(v * r * r + EPS)


def _gelu(x):
    c = np.float32(np.sqrt(2.0 / np.pi))
    return 0.5 * x * (1.0 + jnp.tanh(c * (x + 0.044715 * (x * x * x))))


def _dot(a, b):
    return jnp.dot(a, b, preferred_element_type=f32)


def _mm(a, tile, nk, nn):
    outs = [None] * nn
    for k in range(nk):
        ak = a[:, k * T:(k + 1) * T]
        for n in range(nn):
            d = _dot(ak, tile(k, n))
            outs[n] = d if outs[n] is None else outs[n] + d
    return outs


def _mm_n(a, tile, nk, nn):
    outs = []
    for n in range(nn):
        acc = None
        for k in range(nk):
            d = _dot(a[:, k * T:(k + 1) * T], tile(k, n))
            acc = d if acc is None else acc + d
        outs.append(acc)
    return outs


def _cat(xs):
    return jnp.concatenate(xs, axis=1)


def kernel(x_hbm, k_hbm, v_hbm, wq_hbm, wo_hbm, w3_hbm, w4_hbm, o_ref,
           kb, vb, wq, wo, w3, w4, qc, ss, es, ls, qbs, os_, x_ref, sems):
    VR = HD // 8 // NC

    def k_copy(g):
        return pltpu.make_async_copy(
            k_hbm.at[pl.ds(GH[g] * DH // 8, GS[g] * DH // 8), pl.ds((SK - W) // 16, W // 16)],
            kb.at[pl.ds(GH[g] * DH // 8, GS[g] * DH // 8)], sems.at[NC + 4 + g])

    regions = [r.split(",") for r in SCHED.split(";")]
    kneed = []
    for items in regions:
        gs = []
        for it in items:
            if it[0] in "vq":
                g = int(it[1:].split(".")[0])
                if not any(g in x for x in kneed) and g not in gs:
                    gs.append(g)
        kneed.append(gs)

    def v_copy(c):
        return pltpu.make_async_copy(
            v_hbm.at[pl.ds(c * VR, VR), pl.ds((SK - W) // 16, W // 16)], vb.at[pl.ds(c * VR, VR)], sems.at[c])

    wq_cp = pltpu.make_async_copy(wq_hbm, wq, sems.at[NC])
    wo_cp = pltpu.make_async_copy(wo_hbm, wo, sems.at[NC + 1])
    w3_cp = pltpu.make_async_copy(w3_hbm, w3, sems.at[NC + 2])
    w4_cp = pltpu.make_async_copy(w4_hbm, w4, sems.at[NC + 3])
    x_cp = pltpu.make_async_copy(x_hbm, x_ref, sems.at[NC + 4 + NG])
    x_cp.start()
    for c in range(NC):
        v_copy(c).start()
    wq_cp.start()
    for gs in kneed:
        for g in gs:
            k_copy(g).start()
    wo_cp.start()
    w3_cp.start()
    w4_cp.start()

    def blk(n):
        row = lax.broadcasted_iota(jnp.int32, (M, n * DH), 0)
        col = lax.broadcasted_iota(jnp.int32, (M, n * DH), 1)
        return (col >= row * DH) & (col < row * DH + DH)
    HB = GH[NA]
    vb32 = vb.bitcast(u32)
    kb32 = kb.bitcast(u32)

    def k_retile(g):
        def body(j, c):
            r = pl.multiple_of(GH[g] * DH // 8 + j * 16, 8)
            for a in range(W // 256):
                xf = kb[pl.ds(r, 16), 16 * a:16 * a + 16, :].astype(f32)
                for b in range(2):
                    y = xf[:, 8 * b:8 * b + 8, :].reshape(8, 16, T).astype(bf16)
                    kb[pl.ds(r + 8 * b, 8), 16 * a:16 * a + 16, :] = y
            return c
        lax.fori_loop(0, GS[g] * DH // T, body, 0)
    ss[...] = jnp.zeros(ss.shape, f32)

    x_cp.wait()
    x0 = jnp.broadcast_to(x_ref[0].astype(f32), (M, D))

    def one_pass(p, x):
        first = p == 0
        never = jnp.full((M, T), p, jnp.int32) == 7

        @pl.when(first)
        def _():
            def chunk(c, carry):
                v_copy(c).wait()

                def tr(j, carry2):
                    r = pl.multiple_of(c * VR + j * 16, 16)
                    for a in range(W // 256):
                        xf = vb[pl.ds(r, 16), 16 * a:16 * a + 16, :].astype(f32)
                        ys = [xf[:, 8 * b:8 * b + 8, :].reshape(T, T).T.astype(bf16) for b in range(2)]
                        for b in range(2):
                            vb[pl.ds(r + 8 * b, 8), 16 * a:16 * a + 16, :] = ys[b].reshape(8, 16, T)
                    return carry2
                lax.fori_loop(0, VR // 16, tr, 0)
                return carry
            lax.fori_loop(0, NC, chunk, 0)
            wq_cp.wait()

        xn = _ln(x).astype(bf16)
        gorder = list(range(NA, NG)) + list(range(NA))
        qb = {}

        def qproj(g):
            r0, nt = GH[g] * DH, GS[g] * DH // T
            q = _mm(xn, lambda k, n: wq[k * T:(k + 1) * T, r0 + n * T:r0 + (n + 1) * T], D // T, nt)
            if g < NA:
                qbs[:, r0:r0 + nt * T] = jnp.where(blk(GS[g]), _cat(q), 0.0).astype(bf16)
            else:
                for n in range(nt):
                    qq = q[n].astype(bf16).astype(f32)
                    c0 = r0 - HB * DH + n * T
                    qc[c0:c0 + T, :] = jnp.broadcast_to(qq[0:1, :], (T, T)).T

        def softmax(g):
            s = ss[g]
            m = jnp.max(s, axis=-1, keepdims=True)
            e = jnp.exp((s - m) * SCALE)
            l = jnp.sum(e, axis=-1, keepdims=True)
            es[g] = e.astype(bf16)
            ls[g] = jnp.broadcast_to(l, (M, T))

        NBK = 8

        def ktile(i, n):
            a, b = n // 2, n % 2
            return pltpu.bitcast(kb32[i + 8 * b:i + 8 * b + 8, 8 * a:8 * a + 8, :].reshape(64, T), bf16)

        def qk_mxu(g, part=None):
            r0, nt = GH[g] * DH, GS[g] * DH // T
            nbs = range(W // T // NBK)
            if part is not None:
                nbs = nbs[2 * part:2 * part + 2]
            for nb in nbs:
                outs = _mm(qbs.at[:, r0:r0 + nt * T],
                           lambda k, n: ktile(r0 // 8 + 16 * k, nb * NBK + n), nt, NBK)
                ss[g, :, nb * NBK * T:(nb + 1) * NBK * T] = _cat(outs)

        link = {"prev": None}

        def qk_vpu(g, hi):
            h = GH[g] + hi
            for sb in range(W // T // SB):
                acc = [None] * SB
                acc2 = [None] * SB
                for r in range(DH // 8):
                    c0 = (h - HB) * DH + 8 * r
                    qv = qc[c0:c0 + 8, :]
                    kk = pltpu.bitcast(kb32[h * DH // 8 + r, 8 * sb:8 * sb + 8, :], bf16).astype(f32)
                    for t in range(SB):
                        xx = kk[8 * t:8 * t + 8, :] * qv
                        if r == 0:
                            acc[t] = xx if link["prev"] is None else jnp.where(never, link["prev"], xx)
                        elif r < N1:
                            acc[t] = acc[t] + xx
                        elif r == N1:
                            acc2[t] = xx
                        else:
                            acc2[t] = acc2[t] + xx
                for t in range(SB):
                    a = acc[t] if acc2[t] is None else acc[t] + acc2[t]
                    red = jnp.sum(a, axis=0, keepdims=True)
                    n = sb * SB + t
                    ss[g, hi:hi + 1, n * T:(n + 1) * T] = red
                if LMODE == 0:
                    link["prev"] = jnp.broadcast_to(red, (M, T))
                else:
                    link["prev"] = acc[SB - 1] if link.get("red") is None else jnp.where(never, link["red"], acc[SB - 1])
                    link["red"] = jnp.broadcast_to(red, (M, T))

        def pv(g, part=None):
            r0, nt = GH[g] * DH, GS[g] * DH // T
            ns = list(range(nt))
            if part is not None:
                ns = ns[3 * part:3 * part + 3]

            def tile(k, n):
                J = r0 // T + ns[n]
                a, b = k // 2, k % 2
                w = vb32[16 * J + 8 * b:16 * J + 8 * b + 8, 8 * a:8 * a + 8, :]
                return pltpu.bitcast(w.reshape(64, T), bf16)
            o = _mm_n(es.at[g], tile, W // T, len(ns))
            inv = 1.0 / ls[g]
            bm = blk(GS[g])
            for i, n in enumerate(ns):
                os_[:, r0 + n * T:r0 + (n + 1) * T] = jnp.where(bm[:, n * T:(n + 1) * T], o[i] * inv, 0.0).astype(bf16)

        one = (p >> 3) + 1

        def region(fn):
            if BARRIER:
                def body(i, c):
                    fn()
                    return c
                lax.fori_loop(0, one, body, 0)
            else:
                fn()

        def run(items):
            def fn():
                link["prev"] = None
                link["red"] = None
                for it in items:
                    kind = it[0]
                    f = [int(v) for v in it[1:].split(".")]
                    g = f[0]
                    if kind == "v":
                        for hi in (range(GS[g]) if len(f) == 1 else f[1:]):
                            qk_vpu(g, hi)
                    elif kind == "q":
                        qk_mxu(*f)
                    elif kind == "s":
                        softmax(g)
                    elif kind == "p":
                        pv(*f)
                    elif kind == "j":
                        qproj(g)
            return fn

        for items, gs in zip(regions, kneed):
            if gs:
                @pl.when(first)
                def _():
                    for g in gs:
                        k_copy(g).wait()
                        if g < NA:
                            k_retile(g)
            region(run(items))

        @pl.when(first)
        def _():
            wo_cp.wait()
        if TAIL:
            softmax(NG - 1)
            c0 = GH[NG - 1] * DH
            nk0 = c0 // T
            acc = _cat(_mm(os_.at[:, 0:c0], lambda k, n: wo[k * T:(k + 1) * T, n * T:(n + 1) * T], nk0, D // T))
            pv(NG - 1)
            acc = acc + _cat(_mm(os_.at[:, c0:HD], lambda k, n: wo[c0 + k * T:c0 + (k + 1) * T, n * T:(n + 1) * T],
                                 HD // T - nk0, D // T))
        else:
            acc = _cat(_mm(os_[...], lambda k, n: wo[k * T:(k + 1) * T, n * T:(n + 1) * T], HD // T, D // T))
        x = x + jnp.sum(acc, axis=0, keepdims=True)
        if LN2:
            x1, h = _ln2(x)
            h = h.astype(bf16)
        else:
            x1 = _ln(x)
            h = _ln(x1).astype(bf16)

        @pl.when(first)
        def _():
            w3_cp.wait()
        h = _gelu(_cat(_mm(h, lambda k, n: w3[k * T:(k + 1) * T, n * T:(n + 1) * T], D // T, F // T))).astype(bf16)

        @pl.when(first)
        def _():
            w4_cp.wait()
        return x + x1 + _cat(_mm(h, lambda k, n: w4[k * T:(k + 1) * T, n * T:(n + 1) * T], F // T, D // T))

    x = lax.fori_loop(0, 2, one_pass, x0)
    o_ref[0] = x[0:1, :].astype(o_ref.dtype)


@jax.jit
def pallas_interleave_layers__sliding_block_cached__mixer_s_mlp__decode_kernel(
    A_x, A_k_cache, A_v_cache, A_wq, A_wo, B_x, B_w1, B_w2, B_w3, B_w4,
):
    del B_x, B_w1, B_w2
    kt = jnp.swapaxes(A_k_cache, 2, 3).reshape(HD // 8, 8, SK // T, T).transpose(0, 2, 1, 3).reshape(HD // 8, SK // 16, T)
    vt = jnp.swapaxes(A_v_cache, 2, 3).reshape(HD // 8, 8, SK // T, T).transpose(0, 2, 1, 3).reshape(HD // 8, SK // 16, T)
    hbm = pl.BlockSpec(memory_space=pltpu.HBM)
    return pl.pallas_call(
        kernel,
        out_shape=jax.ShapeDtypeStruct((1, 1, D), bf16),
        in_specs=[hbm] * 7,
        out_specs=pl.BlockSpec(memory_space=pltpu.VMEM),
        scratch_shapes=[
            pltpu.VMEM((HD // 8, W // 16, T), bf16),
            pltpu.VMEM((HD // 8, W // 16, T), bf16),
            pltpu.VMEM((D, HD), bf16),
            pltpu.VMEM((HD, D), bf16),
            pltpu.VMEM((D, F), bf16),
            pltpu.VMEM((F, D), bf16),
            pltpu.VMEM(((H - GH[NA]) * DH, T), f32),
            pltpu.VMEM((NG, M, W), f32),
            pltpu.VMEM((NG, M, W), bf16),
            pltpu.VMEM((NG, M, T), f32),
            pltpu.VMEM((M, GH[NA] * DH), bf16),
            pltpu.VMEM((M, HD), bf16),
            pltpu.VMEM((1, 1, D), bf16),
            pltpu.SemaphoreType.DMA((NC + 5 + NG,)),
        ],
        compiler_params=pltpu.CompilerParams(vmem_limit_bytes=126 * 1024 * 1024),
    )(A_x, kt, vt, A_wq, A_wo, B_w3, B_w4)
```

```python
import jax
import jax.numpy as jnp
import numpy as np
from jax import lax
import jax.experimental.pallas as pl
import jax.experimental.pallas.tpu as pltpu

H, DH, SK, W, D, F = 32, 192, 32768, 4096, 640, 1536
HD = H * DH
M = 8
T = 128
NC = 4
EPS = 1e-5
SCALE = DH ** -0.5
GS = [int(v) for v in "8,4,8,8,4".split(",")]
NA = int("2")
N1 = int("18")
SCHED = "j2,j3,j4,j0,j1;v2.0.1.2.3,q0;s0,v2.4.5.6.7,q1,p0.0,p0.1;s1,s2,v3.0.1.2.3,p0.2,p0.3,p1;v3.4.5.6.7,p2;s3,v4,p3"
NG = len(GS)
GH = [sum(GS[:i]) for i in range(NG)]
HB = GH[NA]
assert sum(GS) == H
f32, bf16, u32 = jnp.float32, jnp.bfloat16, jnp.uint32


def _ln2(x):
    m = jnp.mean(x, axis=-1, keepdims=True)
    xc = x - m
    v = jnp.mean(xc * xc, axis=-1, keepdims=True)
    r = lax.rsqrt(v + EPS)
    x1 = xc * r
    return x1, x1 * lax.rsqrt(v * r * r + EPS)


def _gelu(x):
    c = np.float32(np.sqrt(2.0 / np.pi))
    return 0.5 * x * (1.0 + jnp.tanh(c * (x + 0.044715 * (x * x * x))))


def _dot(a, b):
    return jnp.dot(a, b, preferred_element_type=f32)


def _mm(a, tile, nk, nn):
    outs = [None] * nn
    for k in range(nk):
        ak = a[:, k * T:(k + 1) * T]
        for n in range(nn):
            d = _dot(ak, tile(k, n))
            outs[n] = d if outs[n] is None else outs[n] + d
    return outs


def _mm_n(a, tile, nk, nn):
    outs = []
    for n in range(nn):
        acc = None
        for k in range(nk):
            d = _dot(a[:, k * T:(k + 1) * T], tile(k, n))
            acc = d if acc is None else acc + d
        outs.append(acc)
    return outs


def _cat(xs):
    return jnp.concatenate(xs, axis=1)


def _blk(n):
    row = lax.broadcasted_iota(jnp.int32, (M, n * DH), 0)
    col = lax.broadcasted_iota(jnp.int32, (M, n * DH), 1)
    return (col >= row * DH) & (col < row * DH + DH)


def kernel(x_hbm, k_hbm, v_hbm, wq_hbm, wo_hbm, w3_hbm, w4_hbm, o_ref,
           kb, vb, wq, wo, w3, w4, qc, ss, es, ls, qbs, ob, xb, sems):
    VR = HD // 8 // NC
    win = pl.ds((SK - W) // 16, W // 16)

    def k_copy(g):
        rows = pl.ds(GH[g] * DH // 8, GS[g] * DH // 8)
        return pltpu.make_async_copy(k_hbm.at[rows, win], kb.at[rows], sems.at[NC + 5 + g])

    def v_copy(c):
        return pltpu.make_async_copy(v_hbm.at[pl.ds(c * VR, VR), win], vb.at[pl.ds(c * VR, VR)], sems.at[c])

    wq_cp = pltpu.make_async_copy(wq_hbm, wq, sems.at[NC])
    wo_cp = pltpu.make_async_copy(wo_hbm, wo, sems.at[NC + 1])
    w3_cp = pltpu.make_async_copy(w3_hbm, w3, sems.at[NC + 2])
    w4_cp = pltpu.make_async_copy(w4_hbm, w4, sems.at[NC + 3])
    x_cp = pltpu.make_async_copy(x_hbm, xb, sems.at[NC + 4])

    regions = [r.split(",") for r in SCHED.split(";")]
    kneed, seen = [], []
    for items in regions:
        gs = []
        for it in items:
            if it[0] in "vq":
                g = int(it[1:].split(".")[0])
                if g not in seen:
                    seen.append(g)
                    gs.append(g)
        kneed.append(gs)

    x_cp.start()
    for c in range(NC):
        v_copy(c).start()
    wq_cp.start()
    for g in seen:
        k_copy(g).start()
    wo_cp.start()
    w3_cp.start()
    w4_cp.start()

    vb32 = vb.bitcast(u32)
    kb32 = kb.bitcast(u32)
    ss[...] = jnp.zeros(ss.shape, f32)

    def v_transpose():
        def chunk(c, carry):
            v_copy(c).wait()

            def tr(j, carry2):
                r = pl.multiple_of(c * VR + j * 16, 16)
                for a in range(W // 256):
                    xf = vb[pl.ds(r, 16), 16 * a:16 * a + 16, :].astype(f32)
                    ys = [xf[:, 8 * b:8 * b + 8, :].reshape(T, T).T.astype(bf16) for b in range(2)]
                    for b in range(2):
                        vb[pl.ds(r + 8 * b, 8), 16 * a:16 * a + 16, :] = ys[b].reshape(8, 16, T)
                return carry2
            lax.fori_loop(0, VR // 16, tr, 0)
            return carry
        lax.fori_loop(0, NC, chunk, 0)

    def k_retile(g):
        def body(j, c):
            r = pl.multiple_of(GH[g] * DH // 8 + j * 16, 8)
            for a in range(W // 256):
                xf = kb[pl.ds(r, 16), 16 * a:16 * a + 16, :].astype(f32)
                for b in range(2):
                    y = xf[:, 8 * b:8 * b + 8, :].reshape(8, 16, T).astype(bf16)
                    kb[pl.ds(r + 8 * b, 8), 16 * a:16 * a + 16, :] = y
            return c
        lax.fori_loop(0, GS[g] * DH // T, body, 0)

    def wtile(ref32, i, n):
        a, b = n // 2, n % 2
        return pltpu.bitcast(ref32[i + 8 * b:i + 8 * b + 8, 8 * a:8 * a + 8, :].reshape(64, T), bf16)

    x_cp.wait()
    x0 = jnp.broadcast_to(xb[0].astype(f32), (M, D))

    def one_pass(p, x):
        first = p == 0
        never = jnp.full((M, T), p, jnp.int32) == 7
        one = (p >> 3) + 1

        @pl.when(first)
        def _():
            v_transpose()
            wq_cp.wait()

        xn = _ln2(x)[0].astype(bf16)
        link = [None]

        def qproj(g):
            r0, nt = GH[g] * DH, GS[g] * DH // T
            q = _mm(xn, lambda k, n: wq[k * T:(k + 1) * T, r0 + n * T:r0 + (n + 1) * T], D // T, nt)
            if g < NA:
                qbs[:, r0:r0 + nt * T] = jnp.where(_blk(GS[g]), _cat(q), 0.0).astype(bf16)
            else:
                for n in range(nt):
                    qq = q[n].astype(bf16).astype(f32)
                    c0 = r0 - HB * DH + n * T
                    qc[c0:c0 + T, :] = jnp.broadcast_to(qq[0:1, :], (T, T)).T

        def softmax(g):
            s = ss[g]
            m = jnp.max(s, axis=-1, keepdims=True)
            e = jnp.exp((s - m) * SCALE)
            es[g] = e.astype(bf16)
            ls[g] = jnp.broadcast_to(jnp.sum(e, axis=-1, keepdims=True), (M, T))

        def qk_mxu(g):
            r0, nt = GH[g] * DH, GS[g] * DH // T
            for nb in range(W // T // 8):
                outs = _mm(qbs.at[:, r0:r0 + nt * T], lambda k, n: wtile(kb32, r0 // 8 + 16 * k, nb * 8 + n), nt, 8)
                ss[g, :, nb * 8 * T:(nb + 1) * 8 * T] = _cat(outs)

        def qk_vpu(g, hi):
            h = GH[g] + hi
            for a in range(W // 256):
                acc, acc2 = [None] * 2, [None] * 2
                for r in range(DH // 8):
                    c0 = (h - HB) * DH + 8 * r
                    qv = qc[c0:c0 + 8, :]
                    kk = pltpu.bitcast(kb32[h * DH // 8 + r, 8 * a:8 * a + 8, :], bf16).astype(f32)
                    for t in range(2):
                        xx = kk[8 * t:8 * t + 8, :] * qv
                        if r == 0:
                            acc[t] = xx if link[0] is None else jnp.where(never, link[0], xx)
                        elif r < N1:
                            acc[t] = acc[t] + xx
                        elif r == N1:
                            acc2[t] = xx
                        else:
                            acc2[t] = acc2[t] + xx
                for t in range(2):
                    tot = acc[t] if acc2[t] is None else acc[t] + acc2[t]
                    red = jnp.sum(tot, axis=0, keepdims=True)
                    ss[g, hi:hi + 1, (2 * a + t) * T:(2 * a + t + 1) * T] = red
                link[0] = jnp.broadcast_to(red, (M, T))

        def pv(g, part=None):
            r0, nt = GH[g] * DH, GS[g] * DH // T
            ns = list(range(nt)) if part is None else list(range(3 * part, 3 * part + 3))
            o = _mm_n(es.at[g], lambda k, n: wtile(vb32, r0 // 8 + 16 * ns[n], k), W // T, len(ns))
            inv = 1.0 / ls[g]
            bm = _blk(GS[g])
            for i, n in enumerate(ns):
                ob[:, r0 + n * T:r0 + (n + 1) * T] = jnp.where(
                    bm[:, n * T:(n + 1) * T], o[i] * inv, 0.0).astype(bf16)

        def run(items):
            def body(i, c):
                link[0] = None
                for it in items:
                    f = [int(v) for v in it[1:].split(".")]
                    if it[0] == "v":
                        for hi in (range(GS[f[0]]) if len(f) == 1 else f[1:]):
                            qk_vpu(f[0], hi)
                    else:
                        {"j": qproj, "q": qk_mxu, "s": softmax, "p": pv}[it[0]](*f)
                return c
            lax.fori_loop(0, one, body, 0)

        for items, gs in zip(regions, kneed):
            if gs:
                @pl.when(first)
                def _():
                    for g in gs:
                        k_copy(g).wait()
                        if g < NA:
                            k_retile(g)
            run(items)

        @pl.when(first)
        def _():
            wo_cp.wait()
        softmax(NG - 1)
        c0 = GH[NG - 1] * DH
        acc = _cat(_mm(ob.at[:, 0:c0], lambda k, n: wo[k * T:(k + 1) * T, n * T:(n + 1) * T], c0 // T, D // T))
        pv(NG - 1)
        acc = acc + _cat(_mm(ob.at[:, c0:HD], lambda k, n: wo[c0 + k * T:c0 + (k + 1) * T, n * T:(n + 1) * T],
                             (HD - c0) // T, D // T))
        x = x + jnp.sum(acc, axis=0, keepdims=True)

        x1, h = _ln2(x)

        @pl.when(first)
        def _():
            w3_cp.wait()
        h = _mm(h.astype(bf16), lambda k, n: w3[k * T:(k + 1) * T, n * T:(n + 1) * T], D // T, F // T)
        h = _gelu(_cat(h)).astype(bf16)

        @pl.when(first)
        def _():
            w4_cp.wait()
        return x + x1 + _cat(_mm(h, lambda k, n: w4[k * T:(k + 1) * T, n * T:(n + 1) * T], F // T, D // T))

    x = lax.fori_loop(0, 2, one_pass, x0)
    o_ref[0] = x[0:1, :].astype(o_ref.dtype)


def _tile_order(c):
    return jnp.swapaxes(c, 2, 3).reshape(HD // 8, 8, SK // T, T).transpose(0, 2, 1, 3).reshape(HD // 8, SK // 16, T)


@jax.jit
def pallas_interleave_layers__sliding_block_cached__mixer_s_mlp__decode_kernel(
    A_x, A_k_cache, A_v_cache, A_wq, A_wo, B_x, B_w1, B_w2, B_w3, B_w4,
):
    del B_x, B_w1, B_w2
    return pl.pallas_call(
        kernel,
        out_shape=jax.ShapeDtypeStruct((1, 1, D), bf16),
        in_specs=[pl.BlockSpec(memory_space=pltpu.HBM)] * 7,
        out_specs=pl.BlockSpec(memory_space=pltpu.VMEM),
        scratch_shapes=[
            pltpu.VMEM((HD // 8, W // 16, T), bf16),
            pltpu.VMEM((HD // 8, W // 16, T), bf16),
            pltpu.VMEM((D, HD), bf16),
            pltpu.VMEM((HD, D), bf16),
            pltpu.VMEM((D, F), bf16),
            pltpu.VMEM((F, D), bf16),
            pltpu.VMEM(((H - HB) * DH, T), f32),
            pltpu.VMEM((NG, M, W), f32),
            pltpu.VMEM((NG, M, W), bf16),
            pltpu.VMEM((NG, M, T), f32),
            pltpu.VMEM((M, HB * DH), bf16),
            pltpu.VMEM((M, HD), bf16),
            pltpu.VMEM((1, 1, D), bf16),
            pltpu.SemaphoreType.DMA((NC + 5 + NG,)),
        ],
        compiler_params=pltpu.CompilerParams(vmem_limit_bytes=126 * 1024 * 1024),
    )(A_x, _tile_order(A_k_cache), _tile_order(A_v_cache), A_wq, A_wo, B_w3, B_w4)
```

```python
import jax
import jax.numpy as jnp
import numpy as np
from jax import lax
import jax.experimental.pallas as pl
import jax.experimental.pallas.tpu as pltpu

H, DH, SK, W, D, F = 32, 192, 32768, 4096, 640, 1536
HD = H * DH
M = 8
T = 128
NC = 4
EPS = 1e-5
SCALE = DH ** -0.5
GS = [int(v) for v in "8,4,8,8,4".split(",")]
NA = int("2")
N1 = int("18")
SCHED = "j2,j3,j4,j0,j1;v2.0.1.2.3,q0;s0,v2.4.5.6.7,q1,p0.0,p0.1;s1,s2,v3.0.1.2.3,p0.2,p0.3,p1;v3.4.5.6.7,p2,o0,o1;s3,v4,p3,o2"
VO = int("3")
NG = len(GS)
GH = [sum(GS[:i]) for i in range(NG)]
HB = GH[NA]
assert sum(GS) == H
f32, bf16, u32 = jnp.float32, jnp.bfloat16, jnp.uint32


def _ln2(x):
    m = jnp.mean(x, axis=-1, keepdims=True)
    xc = x - m
    v = jnp.mean(xc * xc, axis=-1, keepdims=True)
    r = lax.rsqrt(v + EPS)
    x1 = xc * r
    return x1, x1 * lax.rsqrt(v * r * r + EPS)


def _gelu(x):
    c = np.float32(np.sqrt(2.0 / np.pi))
    return 0.5 * x * (1.0 + jnp.tanh(c * (x + 0.044715 * (x * x * x))))


def _dot(a, b):
    return jnp.dot(a, b, preferred_element_type=f32)


def _mm(a, tile, nk, nn):
    outs = [None] * nn
    for k in range(nk):
        ak = a[:, k * T:(k + 1) * T]
        for n in range(nn):
            d = _dot(ak, tile(k, n))
            outs[n] = d if outs[n] is None else outs[n] + d
    return outs


def _mm_n(a, tile, nk, nn):
    outs = []
    for n in range(nn):
        acc = None
        for k in range(nk):
            d = _dot(a[:, k * T:(k + 1) * T], tile(k, n))
            acc = d if acc is None else acc + d
        outs.append(acc)
    return outs


def _cat(xs):
    return jnp.concatenate(xs, axis=1)


def _blk(n):
    row = lax.broadcasted_iota(jnp.int32, (M, n * DH), 0)
    col = lax.broadcasted_iota(jnp.int32, (M, n * DH), 1)
    return (col >= row * DH) & (col < row * DH + DH)


def kernel(x_hbm, k_hbm, v_hbm, wq_hbm, wo_hbm, w3_hbm, w4_hbm, o_ref,
           kb, vb, wq, wo, w3, w4, qc, ss, es, ls, qbs, ob, oc, xb, sems):
    VR = HD // 8 // NC
    win = pl.ds((SK - W) // 16, W // 16)

    def k_copy(g):
        rows = pl.ds(GH[g] * DH // 8, GS[g] * DH // 8)
        return pltpu.make_async_copy(k_hbm.at[rows, win], kb.at[rows], sems.at[NC + 5 + g])

    def v_copy(c):
        return pltpu.make_async_copy(v_hbm.at[pl.ds(c * VR, VR), win], vb.at[pl.ds(c * VR, VR)], sems.at[c])

    wq_cp = pltpu.make_async_copy(wq_hbm, wq, sems.at[NC])
    wo_cp = pltpu.make_async_copy(wo_hbm, wo, sems.at[NC + 1])
    w3_cp = pltpu.make_async_copy(w3_hbm, w3, sems.at[NC + 2])
    w4_cp = pltpu.make_async_copy(w4_hbm, w4, sems.at[NC + 3])
    x_cp = pltpu.make_async_copy(x_hbm, xb, sems.at[NC + 4])

    regions = [r.split(",") for r in SCHED.split(";")]
    kneed, seen = [], []
    for items in regions:
        gs = []
        for it in items:
            if it[0] in "vq":
                g = int(it[1:].split(".")[0])
                if g not in seen:
                    seen.append(g)
                    gs.append(g)
        kneed.append(gs)

    x_cp.start()
    for c in range(NC):
        v_copy(c).start()
    wq_cp.start()
    for g in seen:
        k_copy(g).start()
    wo_cp.start()
    w3_cp.start()
    w4_cp.start()

    vb32 = vb.bitcast(u32)
    kb32 = kb.bitcast(u32)
    ss[...] = jnp.zeros(ss.shape, f32)

    def v_transpose():
        def chunk(c, carry):
            v_copy(c).wait()

            def tr(j, carry2):
                r = pl.multiple_of(c * VR + j * 16, 16)
                for a in range(W // 256):
                    xf = vb[pl.ds(r, 16), 16 * a:16 * a + 16, :].astype(f32)
                    ys = [xf[:, 8 * b:8 * b + 8, :].reshape(T, T).T.astype(bf16) for b in range(2)]
                    for b in range(2):
                        vb[pl.ds(r + 8 * b, 8), 16 * a:16 * a + 16, :] = ys[b].reshape(8, 16, T)
                return carry2
            lax.fori_loop(0, VR // 16, tr, 0)
            return carry
        lax.fori_loop(0, NC, chunk, 0)

    def k_retile(g):
        def body(j, c):
            r = pl.multiple_of(GH[g] * DH // 8 + j * 16, 8)
            for a in range(W // 256):
                xf = kb[pl.ds(r, 16), 16 * a:16 * a + 16, :].astype(f32)
                for b in range(2):
                    y = xf[:, 8 * b:8 * b + 8, :].reshape(8, 16, T).astype(bf16)
                    kb[pl.ds(r + 8 * b, 8), 16 * a:16 * a + 16, :] = y
            return c
        lax.fori_loop(0, GS[g] * DH // T, body, 0)

    def wtile(ref32, i, n):
        a, b = n // 2, n % 2
        return pltpu.bitcast(ref32[i + 8 * b:i + 8 * b + 8, 8 * a:8 * a + 8, :].reshape(64, T), bf16)

    x_cp.wait()
    x0 = jnp.broadcast_to(xb[0].astype(f32), (M, D))

    def one_pass(p, x):
        first = p == 0
        never = jnp.full((M, T), p, jnp.int32) == 7
        one = (p >> 3) + 1

        @pl.when(first)
        def _():
            v_transpose()
            wq_cp.wait()

        xn = _ln2(x)[0].astype(bf16)
        link = [None]

        def qproj(g):
            r0, nt = GH[g] * DH, GS[g] * DH // T
            q = _mm(xn, lambda k, n: wq[k * T:(k + 1) * T, r0 + n * T:r0 + (n + 1) * T], D // T, nt)
            if g < NA:
                qbs[:, r0:r0 + nt * T] = jnp.where(_blk(GS[g]), _cat(q), 0.0).astype(bf16)
            else:
                for n in range(nt):
                    qq = q[n].astype(bf16).astype(f32)
                    c0 = r0 - HB * DH + n * T
                    qc[c0:c0 + T, :] = jnp.broadcast_to(qq[0:1, :], (T, T)).T

        def softmax(g):
            s = ss[g]
            m = jnp.max(s, axis=-1, keepdims=True)
            e = jnp.exp((s - m) * SCALE)
            es[g] = e.astype(bf16)
            ls[g] = jnp.broadcast_to(jnp.sum(e, axis=-1, keepdims=True), (M, T))

        def qk_mxu(g):
            r0, nt = GH[g] * DH, GS[g] * DH // T
            for nb in range(W // T // 8):
                outs = _mm(qbs.at[:, r0:r0 + nt * T], lambda k, n: wtile(kb32, r0 // 8 + 16 * k, nb * 8 + n), nt, 8)
                ss[g, :, nb * 8 * T:(nb + 1) * 8 * T] = _cat(outs)

        def qk_vpu(g, hi):
            h = GH[g] + hi
            for a in range(W // 256):
                acc, acc2 = [None] * 2, [None] * 2
                for r in range(DH // 8):
                    c0 = (h - HB) * DH + 8 * r
                    qv = qc[c0:c0 + 8, :]
                    kk = pltpu.bitcast(kb32[h * DH // 8 + r, 8 * a:8 * a + 8, :], bf16).astype(f32)
                    for t in range(2):
                        xx = kk[8 * t:8 * t + 8, :] * qv
                        if r == 0:
                            acc[t] = xx if link[0] is None else jnp.where(never, link[0], xx)
                        elif r < N1:
                            acc[t] = acc[t] + xx
                        elif r == N1:
                            acc2[t] = xx
                        else:
                            acc2[t] = acc2[t] + xx
                for t in range(2):
                    tot = acc[t] if acc2[t] is None else acc[t] + acc2[t]
                    red = jnp.sum(tot, axis=0, keepdims=True)
                    ss[g, hi:hi + 1, (2 * a + t) * T:(2 * a + t + 1) * T] = red
                link[0] = jnp.broadcast_to(red, (M, T))

        def pv(g, part=None):
            r0, nt = GH[g] * DH, GS[g] * DH // T
            ns = list(range(nt)) if part is None else list(range(3 * part, 3 * part + 3))
            o = _mm_n(es.at[g], lambda k, n: wtile(vb32, r0 // 8 + 16 * ns[n], k), W // T, len(ns))
            inv = 1.0 / ls[g]
            bm = _blk(GS[g])
            for i, n in enumerate(ns):
                ob[:, r0 + n * T:r0 + (n + 1) * T] = jnp.where(
                    bm[:, n * T:(n + 1) * T], o[i] * inv, 0.0).astype(bf16)

        def ocol(g):
            r0 = GH[g] * DH
            for n in range(GS[g] * DH // T):
                o = jnp.sum(ob[:, r0 + n * T:r0 + (n + 1) * T].astype(f32), axis=0, keepdims=True)
                oc[r0 + n * T:r0 + (n + 1) * T, :] = jnp.broadcast_to(o, (T, T)).T

        def wo_vpu():
            nr = GH[VO] * DH // 8
            outs, prev = [], None
            for c in range(3):
                acc = [None] * 2
                for r in range(nr if c < 2 else nr // 2):
                    if c < 2:
                        w = wo[8 * r:8 * r + 8, 256 * c:256 * c + 256].astype(f32)
                        ov = oc[8 * r:8 * r + 8, :]
                        xs = [w[:, :T] * ov, w[:, T:] * ov]
                    else:
                        xs = [wo[8 * q:8 * q + 8, 512:640].astype(f32) * oc[8 * q:8 * q + 8, :]
                              for q in (r, r + nr // 2)]
                    for t in range(2):
                        if r == 0:
                            acc[t] = xs[t] if prev is None else jnp.where(never, prev, xs[t])
                        else:
                            acc[t] = acc[t] + xs[t]
                prev = acc[1]
                outs += acc if c < 2 else [acc[0] + acc[1]]
            return _cat(outs)

        def run(items):
            def body(i, c):
                link[0] = None
                for it in items:
                    f = [int(v) for v in it[1:].split(".")]
                    if it[0] == "v":
                        for hi in (range(GS[f[0]]) if len(f) == 1 else f[1:]):
                            qk_vpu(f[0], hi)
                    else:
                        {"j": qproj, "q": qk_mxu, "s": softmax, "p": pv, "o": ocol}[it[0]](*f)
                return c
            lax.fori_loop(0, one, body, 0)

        for items, gs in zip(regions, kneed):
            if gs:
                @pl.when(first)
                def _():
                    for g in gs:
                        k_copy(g).wait()
                        if g < NA:
                            k_retile(g)
            run(items)

        @pl.when(first)
        def _():
            wo_cp.wait()
        softmax(NG - 1)
        c0 = GH[NG - 1] * DH
        b0 = GH[VO] * DH
        acc = _cat(_mm(ob.at[:, b0:c0], lambda k, n: wo[b0 + k * T:b0 + (k + 1) * T, n * T:(n + 1) * T],
                       (c0 - b0) // T, D // T))
        if VO:
            acc = acc + wo_vpu()
        pv(NG - 1)
        acc = acc + _cat(_mm(ob.at[:, c0:HD], lambda k, n: wo[c0 + k * T:c0 + (k + 1) * T, n * T:(n + 1) * T],
                             (HD - c0) // T, D // T))
        x = x + jnp.sum(acc, axis=0, keepdims=True)

        x1, h = _ln2(x)

        @pl.when(first)
        def _():
            w3_cp.wait()
        h = _mm(h.astype(bf16), lambda k, n: w3[k * T:(k + 1) * T, n * T:(n + 1) * T], D // T, F // T)
        h = _gelu(_cat(h)).astype(bf16)

        @pl.when(first)
        def _():
            w4_cp.wait()
        return x + x1 + _cat(_mm(h, lambda k, n: w4[k * T:(k + 1) * T, n * T:(n + 1) * T], F // T, D // T))

    x = lax.fori_loop(0, 2, one_pass, x0)
    o_ref[0] = x[0:1, :].astype(o_ref.dtype)


def _tile_order(c):
    return jnp.swapaxes(c, 2, 3).reshape(HD // 8, 8, SK // T, T).transpose(0, 2, 1, 3).reshape(HD // 8, SK // 16, T)


@jax.jit
def pallas_interleave_layers__sliding_block_cached__mixer_s_mlp__decode_kernel(
    A_x, A_k_cache, A_v_cache, A_wq, A_wo, B_x, B_w1, B_w2, B_w3, B_w4,
):
    del B_x, B_w1, B_w2
    return pl.pallas_call(
        kernel,
        out_shape=jax.ShapeDtypeStruct((1, 1, D), bf16),
        in_specs=[pl.BlockSpec(memory_space=pltpu.HBM)] * 7,
        out_specs=pl.BlockSpec(memory_space=pltpu.VMEM),
        scratch_shapes=[
            pltpu.VMEM((HD // 8, W // 16, T), bf16),
            pltpu.VMEM((HD // 8, W // 16, T), bf16),
            pltpu.VMEM((D, HD), bf16),
            pltpu.VMEM((HD, D), bf16),
            pltpu.VMEM((D, F), bf16),
            pltpu.VMEM((F, D), bf16),
            pltpu.VMEM(((H - HB) * DH, T), f32),
            pltpu.VMEM((NG, M, W), f32),
            pltpu.VMEM((NG, M, W), bf16),
            pltpu.VMEM((NG, M, T), f32),
            pltpu.VMEM((M, HB * DH), bf16),
            pltpu.VMEM((M, HD), bf16),
            pltpu.VMEM((max(GH[VO], 1) * DH, T), f32),
            pltpu.VMEM((1, 1, D), bf16),
            pltpu.SemaphoreType.DMA((NC + 5 + NG,)),
        ],
        compiler_params=pltpu.CompilerParams(vmem_limit_bytes=126 * 1024 * 1024),
    )(A_x, _tile_order(A_k_cache), _tile_order(A_v_cache), A_wq, A_wo, B_w3, B_w4)
```

```python
import jax
import jax.numpy as jnp
import numpy as np
from jax import lax
import jax.experimental.pallas as pl
import jax.experimental.pallas.tpu as pltpu

H, DH, SK, W, D, F = 32, 192, 32768, 4096, 640, 1536
HD = H * DH
M = 8
T = 128
NC = 4
EPS = 1e-5
SCALE = DH ** -0.5
GS = [int(v) for v in "8,4,8,8,4".split(",")]
NA = int("2")
N1 = int("18")
SCHED = "J1,j2,j3,j4,j0;v2.0.1.2.3,q0;s0,v2.4.5.6.7,q1,p0.0,p0.1;s1,s2,v3.0.1.2.3,p0.2,p0.3,p1;v3.4.5.6.7,p2,o0,o1;s3,v4,p3,o2"
VO = int("3")
NG = len(GS)
GH = [sum(GS[:i]) for i in range(NG)]
HB = GH[NA]
assert sum(GS) == H
f32, bf16, u32 = jnp.float32, jnp.bfloat16, jnp.uint32


def _ln2(x):
    m = jnp.mean(x, axis=-1, keepdims=True)
    xc = x - m
    v = jnp.mean(xc * xc, axis=-1, keepdims=True)
    r = lax.rsqrt(v + EPS)
    x1 = xc * r
    return x1, x1 * lax.rsqrt(v * r * r + EPS)


def _gelu(x):
    c = np.float32(np.sqrt(2.0 / np.pi))
    return 0.5 * x * (1.0 + jnp.tanh(c * (x + 0.044715 * (x * x * x))))


def _dot(a, b):
    return jnp.dot(a, b, preferred_element_type=f32)


def _mm(a, tile, nk, nn):
    outs = [None] * nn
    for k in range(nk):
        ak = a[:, k * T:(k + 1) * T]
        for n in range(nn):
            d = _dot(ak, tile(k, n))
            outs[n] = d if outs[n] is None else outs[n] + d
    return outs


def _mm_n(a, tile, nk, nn):
    outs = []
    for n in range(nn):
        acc = None
        for k in range(nk):
            d = _dot(a[:, k * T:(k + 1) * T], tile(k, n))
            acc = d if acc is None else acc + d
        outs.append(acc)
    return outs


def _cat(xs):
    return jnp.concatenate(xs, axis=1)


def _blk(n):
    row = lax.broadcasted_iota(jnp.int32, (M, n * DH), 0)
    col = lax.broadcasted_iota(jnp.int32, (M, n * DH), 1)
    return (col >= row * DH) & (col < row * DH + DH)


def kernel(x_hbm, k_hbm, v_hbm, wq_hbm, wo_hbm, w3_hbm, w4_hbm, o_ref,
           kb, vb, wq, wo, w3, w4, qc, ss, es, ls, qbs, ob, oc, xc_, xb, sems):
    VR = HD // 8 // NC
    win = pl.ds((SK - W) // 16, W // 16)

    def k_copy(g):
        rows = pl.ds(GH[g] * DH // 8, GS[g] * DH // 8)
        return pltpu.make_async_copy(k_hbm.at[rows, win], kb.at[rows], sems.at[NC + 5 + g])

    def v_copy(c):
        return pltpu.make_async_copy(v_hbm.at[pl.ds(c * VR, VR), win], vb.at[pl.ds(c * VR, VR)], sems.at[c])

    wq_cp = pltpu.make_async_copy(wq_hbm, wq, sems.at[NC])
    wo_cp = pltpu.make_async_copy(wo_hbm, wo, sems.at[NC + 1])
    w3_cp = pltpu.make_async_copy(w3_hbm, w3, sems.at[NC + 2])
    w4_cp = pltpu.make_async_copy(w4_hbm, w4, sems.at[NC + 3])
    x_cp = pltpu.make_async_copy(x_hbm, xb, sems.at[NC + 4])

    regions = [r.split(",") for r in SCHED.split(";")]
    kneed, seen = [], []
    for items in regions:
        gs = []
        for it in items:
            if it[0] in "vq":
                g = int(it[1:].split(".")[0])
                if g not in seen:
                    seen.append(g)
                    gs.append(g)
        kneed.append(gs)

    x_cp.start()
    for c in range(NC):
        v_copy(c).start()
    wq_cp.start()
    for g in seen:
        k_copy(g).start()
    wo_cp.start()
    w3_cp.start()
    w4_cp.start()

    vb32 = vb.bitcast(u32)
    kb32 = kb.bitcast(u32)
    ss[...] = jnp.zeros(ss.shape, f32)

    def v_transpose():
        def chunk(c, carry):
            v_copy(c).wait()

            def tr(j, carry2):
                r = pl.multiple_of(c * VR + j * 16, 16)
                for a in range(W // 256):
                    xf = vb[pl.ds(r, 16), 16 * a:16 * a + 16, :].astype(f32)
                    ys = [xf[:, 8 * b:8 * b + 8, :].reshape(T, T).T.astype(bf16) for b in range(2)]
                    for b in range(2):
                        vb[pl.ds(r + 8 * b, 8), 16 * a:16 * a + 16, :] = ys[b].reshape(8, 16, T)
                return carry2
            lax.fori_loop(0, VR // 16, tr, 0)
            return carry
        lax.fori_loop(0, NC, chunk, 0)

    def k_retile(g):
        def body(j, c):
            r = pl.multiple_of(GH[g] * DH // 8 + j * 16, 8)
            for a in range(W // 256):
                xf = kb[pl.ds(r, 16), 16 * a:16 * a + 16, :].astype(f32)
                for b in range(2):
                    y = xf[:, 8 * b:8 * b + 8, :].reshape(8, 16, T).astype(bf16)
                    kb[pl.ds(r + 8 * b, 8), 16 * a:16 * a + 16, :] = y
            return c
        lax.fori_loop(0, GS[g] * DH // T, body, 0)

    def wtile(ref32, i, n):
        a, b = n // 2, n % 2
        return pltpu.bitcast(ref32[i + 8 * b:i + 8 * b + 8, 8 * a:8 * a + 8, :].reshape(64, T), bf16)

    x_cp.wait()
    x0 = jnp.broadcast_to(xb[0].astype(f32), (M, D))

    def one_pass(p, x):
        first = p == 0
        never = jnp.full((M, T), p, jnp.int32) == 7
        one = (p >> 3) + 1

        @pl.when(first)
        def _():
            v_transpose()
            wq_cp.wait()

        xn = _ln2(x)[0].astype(bf16)
        link = [None]

        def qproj(g):
            r0, nt = GH[g] * DH, GS[g] * DH // T
            q = _mm(xn, lambda k, n: wq[k * T:(k + 1) * T, r0 + n * T:r0 + (n + 1) * T], D // T, nt)
            if g < NA:
                qbs[:, r0:r0 + nt * T] = jnp.where(_blk(GS[g]), _cat(q), 0.0).astype(bf16)
            else:
                for n in range(nt):
                    qq = q[n].astype(bf16).astype(f32)
                    c0 = r0 - HB * DH + n * T
                    qc[c0:c0 + T, :] = jnp.broadcast_to(qq[0:1, :], (T, T)).T

        def qproj_vpu(g):
            r0, nt = GH[g] * DH, GS[g] * DH // T
            xf = xn.astype(f32)
            for k in range(D // T):
                xc_[k * T:(k + 1) * T, :] = jnp.broadcast_to(xf[0:1, k * T:(k + 1) * T], (T, T)).T
            outs, prev = [], None
            for c in range(nt // 2):
                acc = [None] * 2
                for r in range(D // 8):
                    w = wq[8 * r:8 * r + 8, r0 + 256 * c:r0 + 256 * c + 256].astype(f32)
                    xv = xc_[8 * r:8 * r + 8, :]
                    for t in range(2):
                        xx = w[:, t * T:(t + 1) * T] * xv
                        if r == 0:
                            acc[t] = xx if prev is None else jnp.where(never, prev, xx)
                        else:
                            acc[t] = acc[t] + xx
                red = [jnp.broadcast_to(jnp.sum(a, axis=0, keepdims=True), (M, T)) for a in acc]
                prev = red[1]
                outs += red
            qbs[:, r0:r0 + nt * T] = jnp.where(_blk(GS[g]), _cat(outs), 0.0).astype(bf16)

        def softmax(g):
            s = ss[g]
            m = jnp.max(s, axis=-1, keepdims=True)
            e = jnp.exp((s - m) * SCALE)
            es[g] = e.astype(bf16)
            ls[g] = jnp.broadcast_to(jnp.sum(e, axis=-1, keepdims=True), (M, T))

        def qk_mxu(g):
            r0, nt = GH[g] * DH, GS[g] * DH // T
            for nb in range(W // T // 8):
                outs = _mm(qbs.at[:, r0:r0 + nt * T], lambda k, n: wtile(kb32, r0 // 8 + 16 * k, nb * 8 + n), nt, 8)
                ss[g, :, nb * 8 * T:(nb + 1) * 8 * T] = _cat(outs)

        def qk_vpu(g, hi):
            h = GH[g] + hi
            for a in range(W // 256):
                acc, acc2 = [None] * 2, [None] * 2
                for r in range(DH // 8):
                    c0 = (h - HB) * DH + 8 * r
                    qv = qc[c0:c0 + 8, :]
                    kk = pltpu.bitcast(kb32[h * DH // 8 + r, 8 * a:8 * a + 8, :], bf16).astype(f32)
                    for t in range(2):
                        xx = kk[8 * t:8 * t + 8, :] * qv
                        if r == 0:
                            acc[t] = xx if link[0] is None else jnp.where(never, link[0], xx)
                        elif r < N1:
                            acc[t] = acc[t] + xx
                        elif r == N1:
                            acc2[t] = xx
                        else:
                            acc2[t] = acc2[t] + xx
                for t in range(2):
                    tot = acc[t] if acc2[t] is None else acc[t] + acc2[t]
                    red = jnp.sum(tot, axis=0, keepdims=True)
                    ss[g, hi:hi + 1, (2 * a + t) * T:(2 * a + t + 1) * T] = red
                link[0] = jnp.broadcast_to(red, (M, T))

        def pv(g, part=None):
            r0, nt = GH[g] * DH, GS[g] * DH // T
            ns = list(range(nt)) if part is None else list(range(3 * part, 3 * part + 3))
            o = _mm_n(es.at[g], lambda k, n: wtile(vb32, r0 // 8 + 16 * ns[n], k), W // T, len(ns))
            inv = 1.0 / ls[g]
            bm = _blk(GS[g])
            for i, n in enumerate(ns):
                ob[:, r0 + n * T:r0 + (n + 1) * T] = jnp.where(
                    bm[:, n * T:(n + 1) * T], o[i] * inv, 0.0).astype(bf16)

        def ocol(g):
            r0 = GH[g] * DH
            for n in range(GS[g] * DH // T):
                o = jnp.sum(ob[:, r0 + n * T:r0 + (n + 1) * T].astype(f32), axis=0, keepdims=True)
                oc[r0 + n * T:r0 + (n + 1) * T, :] = jnp.broadcast_to(o, (T, T)).T

        def wo_vpu():
            nr = GH[VO] * DH // 8
            outs, prev = [], None
            for c in range(3):
                acc = [None] * 2
                for r in range(nr if c < 2 else nr // 2):
                    if c < 2:
                        w = wo[8 * r:8 * r + 8, 256 * c:256 * c + 256].astype(f32)
                        ov = oc[8 * r:8 * r + 8, :]
                        xs = [w[:, :T] * ov, w[:, T:] * ov]
                    else:
                        xs = [wo[8 * q:8 * q + 8, 512:640].astype(f32) * oc[8 * q:8 * q + 8, :]
                              for q in (r, r + nr // 2)]
                    for t in range(2):
                        if r == 0:
                            acc[t] = xs[t] if prev is None else jnp.where(never, prev, xs[t])
                        else:
                            acc[t] = acc[t] + xs[t]
                prev = acc[1]
                outs += acc if c < 2 else [acc[0] + acc[1]]
            return _cat(outs)

        def run(items):
            def body(i, c):
                link[0] = None
                for it in items:
                    f = [int(v) for v in it[1:].split(".")]
                    if it[0] == "v":
                        for hi in (range(GS[f[0]]) if len(f) == 1 else f[1:]):
                            qk_vpu(f[0], hi)
                    else:
                        {"j": qproj, "J": qproj_vpu, "q": qk_mxu, "s": softmax, "p": pv, "o": ocol}[it[0]](*f)
                return c
            lax.fori_loop(0, one, body, 0)

        for items, gs in zip(regions, kneed):
            if gs:
                @pl.when(first)
                def _():
                    for g in gs:
                        k_copy(g).wait()
                        if g < NA:
                            k_retile(g)
            run(items)

        @pl.when(first)
        def _():
            wo_cp.wait()
        softmax(NG - 1)
        c0 = GH[NG - 1] * DH
        b0 = GH[VO] * DH
        acc = _cat(_mm(ob.at[:, b0:c0], lambda k, n: wo[b0 + k * T:b0 + (k + 1) * T, n * T:(n + 1) * T],
                       (c0 - b0) // T, D // T))
        if VO:
            acc = acc + wo_vpu()
        pv(NG - 1)
        acc = acc + _cat(_mm(ob.at[:, c0:HD], lambda k, n: wo[c0 + k * T:c0 + (k + 1) * T, n * T:(n + 1) * T],
                             (HD - c0) // T, D // T))
        x = x + jnp.sum(acc, axis=0, keepdims=True)

        x1, h = _ln2(x)

        @pl.when(first)
        def _():
            w3_cp.wait()
        h = _mm(h.astype(bf16), lambda k, n: w3[k * T:(k + 1) * T, n * T:(n + 1) * T], D // T, F // T)
        h = _gelu(_cat(h)).astype(bf16)

        @pl.when(first)
        def _():
            w4_cp.wait()
        return x + x1 + _cat(_mm(h, lambda k, n: w4[k * T:(k + 1) * T, n * T:(n + 1) * T], F // T, D // T))

    x = lax.fori_loop(0, 2, one_pass, x0)
    o_ref[0] = x[0:1, :].astype(o_ref.dtype)


def _tile_order(c):
    return jnp.swapaxes(c, 2, 3).reshape(HD // 8, 8, SK // T, T).transpose(0, 2, 1, 3).reshape(HD // 8, SK // 16, T)


@jax.jit
def pallas_interleave_layers__sliding_block_cached__mixer_s_mlp__decode_kernel(
    A_x, A_k_cache, A_v_cache, A_wq, A_wo, B_x, B_w1, B_w2, B_w3, B_w4,
):
    del B_x, B_w1, B_w2
    return pl.pallas_call(
        kernel,
        out_shape=jax.ShapeDtypeStruct((1, 1, D), bf16),
        in_specs=[pl.BlockSpec(memory_space=pltpu.HBM)] * 7,
        out_specs=pl.BlockSpec(memory_space=pltpu.VMEM),
        scratch_shapes=[
            pltpu.VMEM((HD // 8, W // 16, T), bf16),
            pltpu.VMEM((HD // 8, W // 16, T), bf16),
            pltpu.VMEM((D, HD), bf16),
            pltpu.VMEM((HD, D), bf16),
            pltpu.VMEM((D, F), bf16),
            pltpu.VMEM((F, D), bf16),
            pltpu.VMEM(((H - HB) * DH, T), f32),
            pltpu.VMEM((NG, M, W), f32),
            pltpu.VMEM((NG, M, W), bf16),
            pltpu.VMEM((NG, M, T), f32),
            pltpu.VMEM((M, HB * DH), bf16),
            pltpu.VMEM((M, HD), bf16),
            pltpu.VMEM((max(GH[VO], 1) * DH, T), f32),
            pltpu.VMEM((D, T), f32),
            pltpu.VMEM((1, 1, D), bf16),
            pltpu.SemaphoreType.DMA((NC + 5 + NG,)),
        ],
        compiler_params=pltpu.CompilerParams(vmem_limit_bytes=126 * 1024 * 1024),
    )(A_x, _tile_order(A_k_cache), _tile_order(A_v_cache), A_wq, A_wo, B_w3, B_w4)
```
